```python
import jax
import jax.numpy as jnp

def _softmax(x, axis=-1):
    return jax.nn.softmax(x, axis=axis)
def _gelu(x):
    return jax.nn.gelu(x, approximate=True)
def _silu(x):
    return jax.nn.silu(x)
def _sigmoid(x):
    return jax.nn.sigmoid(x)
def _layernorm(x, axis=-1, eps=1e-5):
    m = jnp.mean(x, axis=axis, keepdims=True)
    v = jnp.var(x, axis=axis, keepdims=True)
    return (x - m) / jnp.sqrt(v + eps)
def _scatter_add(tgt, idx, src, axis=0):
    return tgt.at[idx].add(src)
def _segment_sum(src, seg, n):
    return jax.ops.segment_sum(src, seg, n)
class _Rng:
    def __init__(self, key):
        self._k = key
    def _next(self):
        self._k, sub = jax.random.split(self._k)
        return sub
    def normal(self, shape):
        return jax.random.normal(self._next(), shape, dtype=jnp.bfloat16)
    def randint(self, lo, hi, shape):
        return jax.random.randint(self._next(), shape, lo, hi, dtype=jnp.int32)
    def uniform(self, shape, lo=0.0, hi=1.0):
        return jax.random.uniform(self._next(), shape, jnp.bfloat16, lo, hi)
    def permutation(self, n):
        return jax.random.permutation(self._next(), n)


kernel_name = 'parallel_sum__sliding_local_dilated__mixer_channel_mlp__prompt'

def _fwd_setup_inputs():
    _rng = _Rng(jax.random.key(int.from_bytes(__import__("os").urandom(4), "little")))
    _w = (lambda a: (lambda t: t.astype(jnp.bfloat16) if jnp.issubdtype(t.dtype, jnp.floating) else t)(jnp.asarray(a)))
    def _A_setup():
        B, S, D = 1, 2048, 576
        return {
            "x": _w((lambda *s: _rng.normal(s) * 0.05)(B, S, D)),
            "wqkv": _w((lambda *s: _rng.normal(s) * 0.05)(D, 3 * D)),
            "wo": _w((lambda *s: _rng.normal(s) * 0.05)(D, D)),
        }
    _A_in = _A_setup()

    def _B_setup():
        B, S, D, F = 1, 2048, 576, 4608
        return {
            "x": _w((lambda *s: _rng.normal(s) * 0.05)(B, S, D)),
            "w1": _w((lambda *s: _rng.normal(s) * 0.05)(D, F) * (D ** -0.5)),
            "b1": _w((lambda *s: _rng.normal(s) * 0.05)(F)),
            "w2": _w((lambda *s: _rng.normal(s) * 0.05)(F, D) * (F ** -0.5)),
            "b2": _w((lambda *s: _rng.normal(s) * 0.05)(D)),
        }
    _B_in = _B_setup()

    return {
        "A_x": _A_in["x"],
        "A_wqkv": _A_in["wqkv"],
        "A_wo": _A_in["wo"],
        "B_x": _B_in["x"],
        "B_w1": _B_in["w1"],
        "B_b1": _B_in["b1"],
        "B_w2": _B_in["w2"],
        "B_b2": _B_in["b2"],
    }

def _fwd_reference(A_x, A_wqkv, A_wo, B_x, B_w1, B_b1, B_w2, B_b2):
    def _A_ref(x, wqkv, wo):
        B, S, D = x.shape
        H = 32; Dh = D // H
        W, dil = 8, 2
        qkv = (lambda x, *d: x.transpose(*d))((x @ wqkv).reshape(B, S, 3, H, Dh), 2, 0, 3, 1, 4)
        q, k, v = qkv[0], qkv[1], qkv[2]
        scale = Dh ** -0.5
        pos = jnp.arange(S)
        off = jnp.arange(W) * dil
        idx = pos[:, None] - off[None, :]
        mask = idx >= 0
        idx_c = jnp.where(mask, idx, 0).reshape(-1)
        kg = k[:, :, idx_c, :].reshape(B, H, S, W, Dh)
        vg = v[:, :, idx_c, :].reshape(B, H, S, W, Dh)
        logits = jnp.einsum("bhsd,bhswd->bhsw", q, kg) * scale
        logits = jnp.where(mask[None, None, :, :], logits, -1e9)
        attn = _softmax(logits, axis=-1)
        o = jnp.einsum("bhsw,bhswd->bhsd", attn, vg)
        return (lambda x, *d: x.transpose(*d))(o, 0, 2, 1, 3).reshape(B, S, D) @ wo

    def _B_ref(x, w1, b1, w2, b2):
        y = _layernorm(x, axis=-1)
        h = _gelu(jnp.einsum("bsd,df->bsf", y, w1) + b1)
        return jnp.einsum("bsf,fd->bsd", h, w2) + b2

    x = A_x
    xn = _layernorm(x, axis=-1)
    return x + _A_ref(xn, A_wqkv, A_wo) + _B_ref(xn, B_w1, B_b1, B_w2, B_b2)


def setup_inputs():
    _inp = _fwd_setup_inputs()
    _gk = jax.random.fold_in(jax.random.key(int.from_bytes(__import__("os").urandom(4), "little")), 2**31 - 1)
    _shapes = [[1, 2048, 576]]
    _dtypes = ['bfloat16']
    _gks = jax.random.split(_gk, len(_shapes))
    _gs = [jax.random.normal(k, s, dtype=jnp.dtype(d)) * 0.05 for k, s, d in zip(_gks, _shapes, _dtypes)]
    _inp["grad_out"] = _gs[0]
    return _inp

def reference(A_x, A_wqkv, A_wo, B_w1, B_b1, B_w2, B_b2, B_x, grad_out):
    _const = dict(B_x=B_x)
    def _f(*_d):
        return _fwd_reference(**{'A_x': _d[0], 'A_wqkv': _d[1], 'A_wo': _d[2], 'B_w1': _d[3], 'B_b1': _d[4], 'B_w2': _d[5], 'B_b2': _d[6], **_const})
    _out, _vjp = jax.vjp(_f, A_x, A_wqkv, A_wo, B_w1, B_b1, B_w2, B_b2)
    _grads = _vjp(grad_out)
    _out0 = jnp.asarray(_out)
    return (_out0, *[jnp.asarray(_g) for _g in _grads])
```

```python
import jax
import jax.numpy as jnp
import jax.experimental.pallas as pl
import jax.experimental.pallas.tpu as pltpu

S, D, F = 2048, 576, 4608
H, HD, W, DIL = 32, 18, 8, 2
EPS = 1e-5
L = 128
TS, FC = 512, 512
TH, FH, DH, DQ = TS // 2, FC // 2, D // 2, D // 4
NT, NF, NL = S // TS, F // FC, S // L
RING = 4
QH = 896
STACK = 49 * DQ + 16
DP = 640
bf16, f32, u32 = jnp.bfloat16, jnp.float32, jnp.uint32
_NN = (((1,), (0,)), ((), ()))
_NT = (((1,), (1,)), ((), ()))
C0 = 0.7978845608028654
C1 = 0.044715
KW = (256, 256, 384, 384, 256, 384, 384)


def _dot(a, b, dims=_NN):
    return jax.lax.dot_general(a, b, dims, preferred_element_type=f32)


def _words(rows, cols):
    return (rows // 2, cols)


def _ld(ref, idx=(), r0=0, n=None, cols=slice(None)):
    rows = slice(None) if n is None else pl.ds(r0 // 2, n // 2)
    return pltpu.bitcast(ref[(*idx, rows, cols)], bf16)


def _pack(v):
    n = v.shape[0] // 2
    return pltpu.bitcast(pltpu.pack_elementwise([v[:n], v[n:]], packed_dtype=bf16), u32)


def _unpack(w):
    w = pltpu.bitcast(w, u32)
    return jnp.concatenate([pltpu.bitcast(w << 16, f32), pltpu.bitcast(w & u32(0xFFFF0000), f32)], 0)


def _split(ref, idx, r0, n):
    return jnp.concatenate([ref[(*idx, pl.ds(r0 + e, n // 2, stride=2))] for e in range(2)], 0)


def _st(ref, idx, r0, v, c0=0):
    ref[(*idx, pl.ds(r0 // 2, v.shape[0] // 2), pl.ds(c0, v.shape[1]))] = _pack(v)


LEFT = ((1, 4), (3, 4), (1,), (4,), (1, 2), (3, -1), (2, -4))
RIGHT = ((1, 4), (1,), (2, -4), (3, -1), (4,), (1, 2), (3, 4))
OUT = ((1, 4, -5, 7), (3, 5), (2, 4), (1, -2, 3, 6))
LEFT_T = ((1, -4), (3, -4), (2, -4), (3, -1), (1, -2), (4,), (1,))
OUT_T = ((1, 6, -5, 3), (7, -5), (2, 6), (2, -1, 7, 4))


def _sum(terms, get):
    v = get(terms[0] - 1)
    for term in terms[1:]:
        v = v + get(term - 1) if term > 0 else v - get(-term - 1)
    return v


def _sums(scheme, xs):
    return [_sum(terms, lambda n: xs[n]) for terms in scheme]


def _sum2(scheme, outer, inner, get):
    return _sum(scheme[outer], lambda a: _sum(scheme[inner], lambda b: get(a, b)))


def _sums2(scheme, outer, get):
    return _sums(scheme, [_sum(scheme[outer], lambda a: get(a, b)) for b in range(4)])


_aset = lambda *x: _sums(LEFT, x)
_bset = lambda *x: _sums(RIGHT, x)
_tset = lambda *x: _sums(LEFT_T, x)
_post = lambda m: _sums(OUT, m)
_tpost = lambda m: _sums(OUT_T, m)


def _weave(main, *sides):
    main = [f for item in main for f in (item if isinstance(item, list) else [item])]
    done = [0] * len(sides)
    if not main:
        return
    for n, item in enumerate(main):
        v = item()
        for s, (pace, side) in enumerate(sides):
            upto = (n + 1) * len(side) // len(main)
            if done[s] < upto and v is not None and pace is not None:
                pace(v())
            while done[s] < upto:
                side[done[s]]()
                done[s] += 1


def _kernel(xT_hbm, gT_hbm, wqkv_hbm, wo_hbm, w1_hbm, w2T_hbm, b1_ref, b2_ref,
            outT_hbm, dxT_hbm, dwqkv_hbm, dwo_hbm, dw1_hbm, db1_ref, dw2T_hbm, db2_ref,
            xb, gb, wqkv_b, wo_b, w_b, dw_b, acc_w, stats, outM, dyM, qkv, oT, dT, db1_s, zero_s, sem_in, sem_w, sem_out):

    def tile_in(src, dst, i, s):
        return pltpu.make_async_copy(src.at[:, pl.ds(i * TS, TS)], dst.at[i, pl.ds(0, D)], sem_in.at[s])

    cp_g = [tile_in(gT_hbm, gb, i, i) for i in range(NT)]
    cp_x = [tile_in(xT_hbm, xb, i, NT + i) for i in range(NT)]
    cp_wo = pltpu.make_async_copy(wo_hbm, wo_b, sem_in.at[2 * NT])
    cp_wqkv = pltpu.make_async_copy(wqkv_hbm, wqkv_b.at[0, pl.ds(0, D)], sem_in.at[2 * NT + 1])

    def cols(j):
        return pl.ds(j * FC if isinstance(j, int) else pl.multiple_of(j * FC, FC), FC)

    def cp_w(j, n):
        slot = n * RING + (j & RING - 1)
        return pltpu.make_async_copy((w1_hbm, w2T_hbm)[n].at[:, cols(j)], w_b.at[slot, pl.ds(0, D)], sem_w.at[slot])

    def cp_dw(j, n):
        slot = 2 * n + (j & 1)
        return pltpu.make_async_copy(dw_b.at[slot], (dw1_hbm, dw2T_hbm)[n].at[:, cols(j)], sem_w.at[2 * RING + slot])

    for c in (cp_wo, cp_g[0]):
        c.start()
    zero_s[0] = 0
    tie = {"z": zero_s[0]}

    def pacer(*refs, slab=0):
        def pace(v):
            for ref in refs:
                w = pltpu.bitcast(v, ref.dtype)
                rows = pl.ds(ref.shape[-2] - w.shape[0], w.shape[0])
                ref[(tie["z"] + slab,) + (0,) * (len(ref.shape) - 3) + (rows, slice(0, L))] = w
        return pace

    def probe(ref, first, r0=0):
        return lambda: ref[tie["z"] + first, pl.ds(r0, 8), pl.ds(0, L)]

    def fenced(main, sides, stops, gate, written):
        legs = [(lo, hi, free) for lo, (hi, free) in zip([0] + [f for _, f in stops], stops)]
        span, done = sum(hi - lo for lo, hi, _ in legs), 0
        for lo, hi, free in legs:
            _weave(main[lo:hi], *[cut(v, done / span, (done + hi - lo) / span) for v in sides])
            _weave(main[hi:free])
            done += hi - lo
            for src in written:
                m = 16 if src.dtype == bf16 else 8
                gate(src[tie["z"], pl.ds(pl.multiple_of(tie["z"], m), m), 0:L])
        _weave(main[stops[-1][1]:])

    def block(body):
        pl.when(tie["z"] == 0)(body)

    def segments(product, rows, store):
        n, held = rows // 4, {}

        def segment(r):
            def run():
                if r == 0:
                    held[0] = product()
                return store(held[0][n * r:n * (r + 1)], pl.ds(n * r, n))
            return run
        return [segment(r) for r in range(4)]

    def cut(stream, a, b):
        pace, todo = stream
        return pace, todo[int(len(todo) * a):int(len(todo) * b)]

    def aligned(v, m):
        return v if isinstance(v, int) else pl.multiple_of(v, m)

    def finish_dw(j, quarter):
        n, r0 = quarter >> 1, aligned((quarter & 1) * (DQ // 2), 8)
        acc = acc_w.at[2 * (j & 1) + n]

        def piece(r, b):
            def run():
                parts = [_sum(OUT[b], lambda m: acc[pl.ds(r0 + (DQ * (7 * k + m) + 8 * r), 8)]) for k in range(7)]
                for a, v in enumerate(_sums(OUT, parts)):
                    dw_b[2 * n + (j & 1), pl.ds(r0 + (DH * (a // 2) + DQ * (b // 2) + 8 * r), 8),
                         pl.ds(FH * (a % 2) + L * (b % 2), L)] = v.astype(bf16)
            return run
        return pacer(acc_w), [piece(r, b) for r in range(DQ // 16) for b in range(4)]

    def normed(x, i, c, twice):
        m1, r1, m2, r2 = [stats[i, n, :, pl.ds(L * c, L)] for n in range(4)]
        xn = (x - m1) * r1
        return (xn - m2) * r2 if twice else xn

    def main_phases(ya, ga, yTa, gTa, wB, b1_s):
        def right_w(j, quarter):
            n, r0 = quarter >> 1, aligned((quarter & 1) * L, L)
            src, dst = w_b.at[n * RING + (j & RING - 1)], wB.at[pl.ds(7 * (2 * (j & 1) + n), 7)]

            def piece(r):
                def run():
                    q = lambda a, c: _unpack(src[pl.ds(r0 + (256 * a + 16 * r), 16), c * FH:(c + 1) * FH])
                    for k, v in enumerate(_bset(q(0, 0), q(0, 1), q(1, 0), q(1, 1))):
                        dst[k, pl.ds(aligned(r0 >> 1, 8) + 8 * r, 8)] = _pack(v)
                return run

            def tail():
                for k, c in ((2, 1), (3, 0), (5, 1), (6, 0)):
                    dst[k, 128:160] = pltpu.bitcast(src[512:576, c * FH:(c + 1) * FH], u32)
                    rows = jax.lax.broadcasted_iota(jnp.int32, (16, FH), 0)
                    b = jnp.broadcast_to(b1_s[j, :, c * FH:(c + 1) * FH], (16, FH))
                    dst[k, 160:168] = _pack(jnp.where(rows < 1 - n, b, 0.0))
            return pacer(w_b), [piece(r) for r in range(L // 16)] + [tail]

        def source(is_x, twice):
            def get(i, r0, n, c, unpack=_unpack):
                v = unpack((xb if is_x else gb)[i, pl.ds(r0, n), pl.ds(L * c, L)])
                return normed(v, i, c, twice) if is_x else v
            return get

        def combos_T(get, dst, i, r):
            st = {}

            def load():
                for a in range(4):
                    for b in range(4):
                        st[a, b] = get(i, DH * (a // 2) + DQ * (b // 2) + 16 * r, 16, 2 * (a % 2) + b % 2)

            def sums(k):
                def run():
                    for n, v in enumerate(_sums2(LEFT, k, lambda a, b: st[a, b])):
                        _st(dst, (i,), DQ * (7 * k + n) + 16 * r, v)
                return run
            return [load] + [sums(k) for k in range(7)]

        def prologue(wP, xB, nat):
            def norm(i, c):
                cs = pl.ds(L * c, L)
                stat = lambda n: stats[i, n, :, cs]
                terms = (lambda x: x, lambda x: jnp.square(x - stat(0)), lambda x: (x - stat(0)) * stat(1),
                         lambda x: jnp.square((x - stat(0)) * stat(1) - stat(2)))

                def sweep(n):
                    def run():
                        total = 0.0
                        for r in range(0, D, 64):
                            v = terms[n](_unpack(xb[i, pl.ds(r, 64), cs]))
                            total = total + sum(v[8 * m:8 * m + 8] for m in range(1, 8)) + v[0:8]
                        mean = jnp.sum(total, 0, keepdims=True) * (1.0 / D)
                        stats[i, n, :, cs] = jax.lax.rsqrt(mean + EPS) if n % 2 else mean
                    return run
                return [sweep(n) for n in range(4)]

            def flip(get, i, c, r, fill):
                def run():
                    n = min(L, D - L * r)
                    v = get(i, L * r, n, c, lambda w: w.astype(f32))
                    if n < L:
                        row = jax.lax.broadcasted_iota(jnp.int32, (L - n, L), 0)
                        v = jnp.concatenate([v, jnp.where(row == 0, fill, 0.0)], 0)
                    nat[r, pl.ds(L * c, L)] = v.T
                return run

            def wide_aset(q):
                blocks = (q(0, 0, 2), q(0, 2, 2), q(1, 0, 2), q(1, 2, 2))
                t1, t2 = q(0, 4, 1), q(1, 4, 1)
                tails = {2: t1, 3: t2, 5: t2 - t1, 6: t1 - t2}
                return [jnp.concatenate([v, tails[k]], 1) if k in tails else v
                        for k, v in enumerate(_aset(*blocks))], blocks, t1 + t2

            def combos_N(dst, i, r, is_g):
                def run():
                    q = lambda half, c0, n: jnp.concatenate(
                        [_split(nat, (c0 + u,), TH * half + 16 * r, 16) for u in range(n)], 1)
                    vs, blocks, tail = wide_aset(q)
                    for k, v in enumerate(vs):
                        _st(dst, (7 * i + k,), 16 * r, v)
                    if is_g:
                        t = jnp.concatenate([blocks[0] + blocks[2], blocks[1] + blocks[3], tail], 1)
                        t = t[0:8] + t[8:16]
                        db1_s[NF] += t[:, 0:FC]
                        db1_s[NF + 1, :, 0:L] += t[:, FC:DP]
                return run

            def layouts(i, is_x):
                get = source(is_x, True)
                return ([flip(get, i, c, r, 1.0 if is_x else 0.0) for c in range(4) for r in range(5)] +
                        [f for r in range(DQ // 16 if is_x else 0) for f in combos_T(get, yTa, i, r)] +
                        [combos_N(ya if is_x else ga, i, r, not is_x) for r in range(TH // 16)])

            def right(i):
                def piece(r, c):
                    return lambda: _st(xB, (i % 2,), 64 * r, source(True, False)(i, 64 * r, 64, c), L * c)
                return [piece(r, c) for r in range(D // 64) for c in range(4)]

            def put_left(part, r, v):
                for e in range(2):
                    wP[part, pl.ds(DH * e + 16 * r, 16), :] = v[16 * e:16 * (e + 1), 0:D].astype(bf16)

            def flip_w(c, r):
                def run():
                    n, m = min(L, 3 * D - L * c), min(L, D - L * r)
                    v = wqkv_b[0, pl.ds(L * r, m), pl.ds(L * c, n)].astype(f32)
                    if n < L:
                        v = jnp.concatenate([v, jnp.zeros((m, L - n), f32)], 1)
                    if m < L:
                        v = jnp.concatenate([v, jnp.zeros((L - m, L), f32)], 0)
                    nat[r, pl.ds(TS + L * c, L)] = v.T
                return run

            def left_w(part):
                def piece(r):
                    return lambda: put_left(part, r, jnp.concatenate(
                        [_split(nat, (u,), TS + D * part + 32 * r, 32) for u in range(5)], 1))
                return [piece(r) for r in range(D // 32)]

            def project(i, part):
                def item(c, e):
                    rows, cs, n = pl.ds(DQ * e, DQ), pl.ds(TH * c, TH), DQ // 3

                    def segment(r, held):
                        def run():
                            if r == 0:
                                rhs = gb[i, 0:D, cs] if part == 3 else _ld(xB, (i % 2,), cols=cs)
                                held.append(_dot(jnp.concatenate(
                                    [wP[part, pl.ds(DH * u + DQ * e, DQ), :] for u in range(2)], 0), rhs))
                            v = jnp.concatenate([held[0][DQ * u + n * r:DQ * u + n * (r + 1)] for u in range(2)], 0)
                            at = DH * part + DQ * e + n * r
                            for u in range(2):
                                qkv[4 * i + 2 * c + u + 1, pl.ds(at, n)] = _pack(v[:, L * u:L * (u + 1)])
                            return probe(qkv, 4 * i + 2 * c + 1, at)
                        return run
                    held = []
                    return [segment(r, held) for r in range(3)]
                return [item(c, e) for c in range(2) for e in range(2)]

            def setup():
                b = b1_ref[...].astype(f32)
                for j in range(NF):
                    b1_s[j] = b[:, FC * j:FC * (j + 1)]
                for k in range(28):
                    wB[k, 160:192, :] = jnp.zeros((32, FH), u32)
                db1_s[...] = jnp.zeros(db1_s.shape, f32)
                for t in (0, NL + 1):
                    qkv[t] = jnp.zeros(qkv.shape[1:], u32)

            later = [cp_g[1], cp_wqkv, cp_x[0], cp_g[2], cp_g[3], cp_x[1], cp_x[2], cp_x[3]]
            later += [cp_w(j, n) for j in range(3) for n in range(2)]
            for c in later[:3]:
                c.start()
            setup()
            cp_wo.wait()
            for r in range(D // 32):
                put_left(3, r, _unpack(wo_b[pl.ds(32 * r, 32), :]))
            cp_g[0].wait()
            pg, px, pw = pacer(gb), pacer(xb), pacer(nat)

            flips = [flip_w(c, r) for c in range(14) for r in range(5)]

            def job(i, part):
                stats_of = lambda m: (px, [f for c in range(4) for f in norm(m, c)] + right(m))
                if part == 3:
                    sides = ([(pg, layouts(0, False))], [(pw, flips[:35])], [(pw, flips[35:])],
                             [stats_of(0), (pw, left_w(0))])[i]
                else:
                    sides = [(pw, left_w(part + 1))] if i == 0 and part < 2 else []
                    if part == 0 and i > 0:
                        sides.append((pg, layouts(i, False)))
                    if part == 1:
                        sides.append((px, layouts(i, True)))
                    if part == 2:
                        sides += [stats_of(i + 1)] if i + 1 < NT else [right_w(0, m) for m in range(4)]
                _weave(project(i, part), *sides)

            for i in range(NT):
                for c in later[3 + 2 * i:5 + 2 * i]:
                    c.start()
                (cp_g[i + 1] if i + 1 < NT else cp_x[0]).wait()
                if i == 1:
                    cp_wqkv.wait()
                block(lambda: job(i, 3))
            for c in later[11:]:
                c.start()
            for i in range(NT):
                for c in [cp_x[i + 1]] if i + 1 < NT else later[8:12]:
                    c.wait()
                block(lambda: [job(i, part) for part in range(3)] and None)

        pl.run_scoped(prologue,
                      pltpu.VMEM((4, D, D), bf16), pltpu.VMEM((2, *_words(D, TS)), u32),
                      pltpu.VMEM((5, TS + 14 * L + 8, L), f32))

        def mlp(wA, mp, md, hB, dB, p_s, dl_s, hd_s):
            tie["z"] = zero_s[0]

            def left_w(j, quarter):
                n, r0 = quarter >> 1, aligned((quarter & 1) * 64, 64)
                src, dst = w_b.at[n * RING + (j & RING - 1)], wA.at[2 * (j & 1) + n]

                def piece(r, k):
                    def run():
                        q = lambda a, b: _unpack(src[pl.ds(r0 + (DH * (a // 2) + DQ * (b // 2) + 16 * r), 16),
                                                     pl.ds(FH * (a % 2) + L * (b % 2), L)])
                        for m, v in enumerate(_sums2(LEFT_T, k, q)):
                            dst[pl.ds(aligned(r0 >> 1, 8) + (DQ // 2 * (7 * k + m) + 8 * r), 8)] = _pack(v)
                    return run
                return pacer(w_b), [piece(r, k) for r in range(5) for k in range(7)]

            def stage_A(n):
                i, j = n & 3, n >> 2

                def item(xa, w, m, k):
                    def store(v, rows):
                        m[2 * k, rows] = v[:, 0:L]
                        m[2 * k + 1, rows] = v[:, L:FH]
                        return probe(m, 2 * k)
                    return segments(lambda: _dot(_ld(xa, (7 * i + k,), cols=slice(0, KW[k])),
                                                 _ld(wB, (7 * (2 * (j & 1) + w) + k,), 0, KW[k])), TH, store)
                return [item(ya, 0, mp, k) for k in range(7)] + [item(ga, 1, md, k) for k in range(7)]

            def stage_G(n):
                def piece(r, c):
                    st = {}

                    def total(m, e):
                        return _post([m[2 * k + c, pl.ds(16 * r + e, 8, stride=2)] for k in range(7)])

                    def act(e):
                        def run():
                            st["h", e], st["g"] = [], []
                            for p in total(mp, e):
                                p2 = p * p
                                a = 0.5 + 0.5 * jnp.tanh(p * (C0 + (C0 * C1) * p2))
                                h = p * a
                                st["h", e].append(h)
                                st["g"].append(a + (h - h * a) * (2 * C0 + (6 * C0 * C1) * p2))
                            if e == 1:
                                emit(hB, "h")
                        return run

                    def grad(e):
                        def run():
                            st["d", e] = [d * g for d, g in zip(total(md, e), st["g"])]
                            if e == 1:
                                emit(dB, "d")
                                for half in range(2):
                                    t = (st["d", 0][half] + st["d", 0][2 + half]) + (st["d", 1][half] + st["d", 1][2 + half])
                                    where = pl.ds(half * FH + L * c, L)
                                    db1_s[n >> 2, :, where] += t
                        return run

                    def emit(dst, name):
                        for q, v in enumerate(zip(st[name, 0], st[name, 1])):
                            at = (r % 8, "hd".index(name), 2 * (r // 8) + c, q)
                            hd_s[at] = jnp.concatenate(v, 0)
                    return [act(0), grad(0), act(1), grad(1)]

                def second(r, w, k):
                    def run():
                        for m, v in enumerate(_sums2(RIGHT, k, lambda a, b: hd_s[r, w, b, a])):
                            _st((hB, dB)[w], (7 * k + m,), 16 * r, v)
                    return run
                return ((pacer(mp, md),
                         [f for r in range(TH // 16) for c in range(2) for f in piece(r, c)]),
                        (pacer(hd_s, slab=8), [second(r, w, k) for w in range(2) for r in range(L // 16) for k in range(7)]))

            def stage_BC(n):
                i, j = n & 3, n >> 2
                plan = (((acc_w, 2 * (j & 1) + 1), i > 0, (gTa, i), hB, _NN),
                        ((acc_w, 2 * (j & 1)), i > 0, (yTa, i), dB, _NN),
                        ((outM, i), j > 0, (wA, 2 * (j & 1) + 1), hB, _NT),
                        ((dyM, i), j > 0, (wA, 2 * (j & 1)), dB, _NT))
                jobs = [(*p, k) for p in plan for k in range(49)]

                def group(four):
                    m, held = DQ // 3, []

                    def segment(r):
                        def run():
                            if r == 0:
                                held.extend(_dot(_ld(a, (at,), DQ * k, DQ), _ld(b, (k,), 0, L), dims)
                                            for _, _, (a, at), b, dims, k in four)
                            old = [jnp.where(started, acc[at, pl.ds(DQ * k + m * r, m)], 0.0)
                                   for (acc, at), started, *_, k in four]
                            for ((acc, at), *_, k), u, v in zip(four, old, held):
                                acc[at, pl.ds(DQ * k + m * r, m)] = u + v[m * r:m * (r + 1)]
                            return probe(acc, at, DQ * k)
                        return run
                    return [segment(r) for r in range(3)]
                return [group(jobs[k:k + 4]) for k in range(0, len(jobs), 4)]

            def attention(t, hg):
                st = {}
                lane = lambda: jax.lax.broadcasted_iota(jnp.int32, (8, L), 1)

                def rows(part, d):
                    return pl.ds((part * D + 8 * HD * hg) // 2 + d, 8, stride=HD // 2)

                def ld(dt, part, d):
                    return qkv[t + 1 + dt, rows(part, d), :]

                def back(cur, prev, w):
                    if w == 0:
                        return cur
                    return pltpu.roll(jnp.where(lane() < L - DIL * w, cur, prev), DIL * w, 1)

                def ahead(cur, nxt, w):
                    if w == 0:
                        return cur
                    return pltpu.roll(jnp.where(lane() >= DIL * w, cur, nxt), L - DIL * w, 1)

                def scores(own, other, dst, d):
                    def run():
                        a, cur, prev = _unpack(ld(0, own, d)), ld(0, other, d), ld(-1, other, d)
                        for w in range(W):
                            v = a * _unpack(back(cur, prev, w))
                            v = v[0:8] + v[8:16]
                            st[w] = v if d == 0 else st[w] + v
                            if d == HD // 2 - 1:
                                dst[t & 3, hg, w] = st[w]
                    return run

                def soft():
                    pos = lane() + t * L
                    lg = [jnp.where(pos >= DIL * w, p_s[t & 3, hg, w] * HD ** -0.5, -1e9) for w in range(W)]
                    m = lg[0]
                    for w in range(1, W):
                        m = jnp.maximum(m, lg[w])
                    e = [jnp.exp(x - m) for x in lg]
                    tot = e[0]
                    for w in range(1, W):
                        tot = tot + e[w]
                    inv = 1.0 / tot
                    p = [x * inv for x in e]
                    dp = [dl_s[t & 3, hg, w] for w in range(W)]
                    c = p[0] * dp[0]
                    for w in range(1, W):
                        c = c + p[w] * dp[w]
                    for w in range(W):
                        p_s[t & 3, hg, w] = p[w]
                        dl_s[t & 3, hg, w] = jnp.where(pos >= DIL * w, p[w] * (dp[w] - c) * HD ** -0.5, 0.0)

                def gather(src, other, dst, part, d):
                    def run():
                        if d == 0:
                            for w in range(W):
                                st[w] = jnp.concatenate([src[t & 3, hg, w]] * 2, 0)
                        cur, prev = ld(0, other, d), ld(-1, other, d)
                        v = st[0] * _unpack(cur)
                        for w in range(1, W):
                            v = v + st[w] * _unpack(back(cur, prev, w))
                        dst[t, rows(part, d), :] = _pack(v)
                    return run

                def scatter(src, other, dst, part, d):
                    def run():
                        if d == 0:
                            for w in range(W):
                                st[w] = jnp.concatenate([ahead(src[t & 3, hg, w], src[(t + 1) & 3, hg, w], w)] * 2, 0)
                        cur, nxt = ld(0, other, d), ld(1, other, d)
                        v = st[0] * _unpack(cur)
                        for w in range(1, W):
                            v = v + st[w] * _unpack(ahead(cur, nxt, w))
                        dst[t, rows(part, d), :] = _pack(v)
                    return run

                ds = range(HD // 2)
                return ([scores(0, 1, p_s, d) for d in ds] + [scores(3, 2, dl_s, d) for d in ds] + [soft] +
                        [gather(p_s, 2, oT, 0, d) for d in ds] + [gather(dl_s, 1, dT, 0, d) for d in ds] +
                        [scatter(dl_s, 0, dT, 1, d) for d in ds] + [scatter(p_s, 3, dT, 2, d) for d in ds])

            for ref in (p_s, dl_s):
                ref[0] = jnp.zeros(ref.shape[1:], f32)

            def wipe(k):
                def run():
                    acc_w[2 + k // 49, pl.ds(DQ * (k % 49), DQ)] = jnp.zeros((DQ, L), f32)
                return run
            rows_g = lambda tiles: (pacer(gb), [f for i in tiles for r in range(DQ // 16)
                                                for f in combos_T(source(False, False), gTa, i, r)])
            block(lambda: _weave(stage_A(0), *[left_w(0, m) for m in range(4)], rows_g((0, 1))))

            def warm_up():
                main, g = stage_A(1), stage_G(0)
                for f in g[0][1]:
                    f()
                _weave(main, g[1], right_w(1, 0), rows_g((2, 3)), (pacer(hB), [wipe(k) for k in range(98)]))
            block(warm_up)

            def step(n, carry):
                tie["z"] = zero_s[0]
                i, j = n & 3, n >> 2

                @pl.when(i == NT - 1)
                def _():
                    for w in range(2):
                        pl.when(j >= 2)(lambda: cp_dw(j - 2, w).wait())
                        pl.when(j + 2 < NF)(lambda: cp_w(j + 2, w).wait())
                        pl.when(j + 3 < NF)(lambda: cp_w(j + 3, w).start())

                @pl.when((i == 0) & (j >= 2))
                def _():
                    for w in range(2):
                        cp_dw(j - 2, w).start()

                m = jnp.minimum(n, 2 * NL - 2 + (n & 1))
                att = (pacer(qkv), [f for u in range(2) for f in attention(NL - 1 - (m >> 1), 2 * (m & 1) + u)])
                g, x = stage_G(n + 1), 0.9
                main = stage_BC(n)
                _weave(main[:-1], g[0], cut(att, 0, x),
                       right_w(jnp.minimum(((n + 1) >> 2) + 1, NF - 1), (n + 1) & 3))
                _weave(main[-1:])
                sides = [g[1], cut(att, x, 1), left_w(jnp.minimum(j + 1, NF - 1), i), finish_dw(j + 1, i)]
                fenced(stage_A(n + 2), sides, ((5, 7), (11, 12)), pacer(ga, slab=NT * 7), (oT, dT, wA, hB, dB, dw_b))
                return carry

            jax.lax.fori_loop(0, NT * NF - 2, step, 0)
            tie["z"] = zero_s[0]


            def drain():
                n = NT * NF - 2
                main, g = stage_BC(n), stage_G(n + 1)
                _weave(main[:40], g[0], finish_dw(NF - 2, 2))
                _weave(main[40:])
                for f in cut(g[1], 0, 0.5)[1]:
                    f()
                main = stage_BC(n + 1)
                _weave(main[:10], cut(g[1], 0.5, 1))
                _weave(main[10:], finish_dw(NF - 2, 3))
            block(drain)
            for w in range(2):
                cp_dw(NF - 3, w).wait()
                cp_dw(NF - 2, w).start()

        V = pltpu.VMEM
        pl.run_scoped(
            mlp, V((4, *_words(STACK, L)), u32), V((14, TH + 8, L), f32), V((14, TH + 8, L), f32),
            V((49, *_words(L + 16, L)), u32), V((49, *_words(L, L)), u32),
            V((4, 4, W, 8, L), f32), V((4, 4, W, 8, L), f32), V((9, 2, 4, 4, 16, L), f32))

    V = pltpu.VMEM
    pl.run_scoped(
        main_phases,
        V((NT * 7 + 1, *_words(TH, 384)), u32), V((NT * 7 + 1, *_words(TH, 384)), u32),
        V((NT, *_words(STACK, L)), u32), V((NT, *_words(STACK, L)), u32),
        V((4 * 7, *_words(384, FH)), u32), V((NF, 1, FC), f32))

    def epilogue(out_b, dx_b, woT, b2c, wT, xA, dS, fin, work, dwo, *accs):
        tie["z"] = zero_s[0]

        def tile_out(src, dst, i, s):
            return pltpu.make_async_copy(src.at[i], dst.at[:, pl.ds(i * TS, TS)], sem_out.at[s])

        cp_out = [tile_out(out_b, outT_hbm, i, i) for i in range(NT)]
        cp_dx = [tile_out(dx_b, dxT_hbm, i, NT + i) for i in range(NT)]
        cp_dwqkv = [pltpu.make_async_copy(wqkv_b.at[0, pl.ds(0, D), pl.ds(c, n)], dwqkv_hbm.at[:, pl.ds(c, n)],
                                          sem_out.at[2 * NT + 1 + m])
                    for m, (c, n) in enumerate(((0, 3 * TH), (3 * TH, 3 * D - 3 * TH)))]
        cp_dwo = pltpu.make_async_copy(wo_b, dwo_hbm, sem_out.at[2 * NT])

        def wide(ref, t, tiles, r0=0, n=None):
            return jnp.concatenate([_ld(ref, (t + u,), r0, n) for u in range(tiles)], 1)

        def flip_wo(c):
            n = min(L, D - L * c)
            v = wo_b[:, pl.ds(L * c, n)].astype(f32)
            b = b2_ref[:, pl.ds(L * c, n)].astype(f32)
            if n < L:
                v = jnp.concatenate([v, jnp.zeros((D, L - n), f32)], 1)
                b = jnp.concatenate([b, jnp.zeros((1, L - n), f32)], 1)
            v = jnp.concatenate([v, jnp.zeros((DP - D, L), f32)], 0)
            woT[pl.ds(L * c, n), :] = v.T[0:n, 0:D].astype(bf16)
            b2c[pl.ds(L * c, n), :] = jnp.broadcast_to(b, (L, L)).T[0:n]

        def left_w(r):
            def run():
                def q(half, c):
                    w = min(QH, 3 * D - QH * c)
                    v = _unpack(wqkv_b[0, pl.ds(DH * half + 16 * r, 16), pl.ds(QH * c, w)])
                    return v if w == QH else jnp.concatenate([v, jnp.zeros((16, QH - w), f32)], 1)
                for k, v in enumerate(_tset(q(0, 0), q(0, 1), q(1, 0), q(1, 1))):
                    _st(wT, (k,), 16 * r, v)
            return run

        def left_x(i, r, u):
            def run():
                q = lambda r0, c: normed(_unpack(xb[i, pl.ds(r0 + 48 * r, 48), pl.ds(L * (2 * c + u), L)]),
                                         i, 2 * c + u, False)
                for k, v in enumerate(_aset(q(0, 0), q(0, 1), q(DH, 0), q(DH, 1))):
                    _st(xA, (k,), 48 * r, v, TH * i + L * u)
            return run

        def right_d(i, r, u):
            def run():
                def q(half, c):
                    if QH * half + 32 * r >= 3 * D:
                        return jnp.zeros((32, L), f32)
                    return _unpack(dT[4 * i + 2 * c + u, pl.ds((QH * half + 32 * r) // 2, 16)])
                for k, v in enumerate(_bset(q(0, 0), q(1, 0), q(0, 1), q(1, 1))):
                    _st(dS, (k,), 32 * r, v, TH * i + L * u)
            return run

        def rights(i):
            return [right_d(i, r, u) for r in range(QH // 32) for u in range(2)]

        def fwd(i, half, a):
            def store(v, rows):
                fin[half, pl.ds(DH * a + rows.start, rows.size)] = v
                return probe(fin, half)
            return segments(lambda: _dot(woT[pl.ds(DH * a, DH), :], wide(oT, 4 * i + 2 * half, 2)), DH, store)

        def fwd_finish(i, r, b):
            def run():
                parts = [_sum(OUT_T[b], lambda n: outM[i, pl.ds(DQ * (7 * k + n) + 8 * r, 8)]) for k in range(7)]
                for a, v in enumerate(_sums(OUT_T, parts)):
                    rows = pl.ds(DH * (a // 2) + DQ * (b // 2) + 8 * r, 8)
                    cs = pl.ds(TH * (a % 2) + L * (b % 2), L)
                    v = v + fin[a % 2, rows, pl.ds(L * (b % 2), L)] + b2c[rows, :] + xb[i, rows, cs].astype(f32)
                    out_b[i, rows, cs] = v.astype(bf16)
            return run

        def bwd(i, acc):
            def item(k):
                def store(v, rows):
                    acc[k, rows] = v
                    return probe(acc, k)
                return segments(lambda: _dot(_ld(wT, (k,)), _ld(dS, (k,), cols=pl.ds(TH * i, TH))), DH, store)
            return [item(k) for k in range(7)]

        def bwd_finish(i, c, acc):
            cs, st, n = pl.ds(L * c, L), {}, 48
            x = lambda r, twice: normed(xb[i, pl.ds(n * r, n), cs].astype(f32), i, c, twice)
            fold = lambda v: sum(v[8 * m:8 * m + 8] for m in range(1, n // 8)) + v[0:8]
            mean = lambda v: jnp.sum(v, 0, keepdims=True) * (1.0 / D)

            def tally(r, name, d, xn):
                work[c % 2, pl.ds(n * r, n)] = d
                s1, s2 = fold(d), fold(d * xn)
                st[name] = (s1, s2) if r == 0 else (st[name][0] + s1, st[name][1] + s2)
                if n * (r + 1) == D:
                    st[name] = [mean(v) for v in st[name]]

            def first(r):
                a, b, r0 = n * r // DH, n * r % DH // DQ, n * r % DQ
                dy = _sum2(OUT_T, 2 * a + c // 2, 2 * b + c % 2, lambda k, m: dyM[i, pl.ds(DQ * (7 * k + m) + r0, n)])
                tally(r, "y", dy, x(r, True))

            def second(r):
                dy, rs = work[c % 2, pl.ds(n * r, n)], pl.ds(n * r % DH, n)
                d = stats[i, 3, :, cs] * (dy - st["y"][0] - x(r, True) * st["y"][1])
                d = d + _sum(OUT_T[2 * (n * r // DH) + c // 2], lambda k: acc[k, rs, pl.ds(L * (c % 2), L)])
                tally(r, "x", d, x(r, False))

            def third(r):
                rs = pl.ds(n * r, n)
                d = stats[i, 1, :, cs] * (work[c % 2, rs] - st["x"][0] - x(r, False) * st["x"][1])
                dx_b[i, rs, cs] = (d + gb[i, rs, cs].astype(f32)).astype(bf16)
            return [lambda f=f, r=r: f(r) for f in (first, second, third) for r in range(D // n)]

        def grad_w(c, n, acc):
            def item(k):
                def store(v, rows):
                    acc[k, rows, 0:n] = v
                    return probe(acc, k)
                return segments(lambda: _dot(_ld(xA, (k,)), _ld(dS, (k,), c, n), _NT), DH, store)

            def finish(r, u):
                def run():
                    for q, v in enumerate(_post([acc[k, pl.ds(16 * r, 16), pl.ds(u, L)] for k in range(7)])):
                        c0 = QH * (q % 2) + c + u
                        w = min(L, 3 * D - c0)
                        wqkv_b[0, pl.ds(DH * (q // 2) + 16 * r, 16), pl.ds(c0, w)] = v[:, 0:w].astype(bf16)
                return run
            return [item(k) for k in range(7)], (pacer(acc), [finish(r, u) for r in range(18) for u in range(0, n, L)])

        for c in range(5):
            flip_wo(c)
        def tile(i):
            _weave([fwd(i, half, a) for half in range(2) for a in range(2)],
                   (pacer(xb), [left_x(i, r, u) for r in range(6) for u in range(2)]), finish_dw(NF - 1, i),
                   (None, [] if i else [left_w(r) for r in range(DH // 16)] + rights(0)))
            _weave(bwd(i, accs[i]), (pacer(dT), rights(i + 1) if i + 1 < NT else []),
                   (pacer(fin, outM), [fwd_finish(i, r, b) for r in range(DQ // 8) for b in range(4)]))

        for i in range(NT):
            block(lambda: tile(i))
            cp_out[i].start()
        for w in range(2):
            cp_dw(NF - 1, w).start()
        grads = [grad_w(c, min(TH, QH - c), accs[NT + n % 2]) for n, c in enumerate(range(0, QH, TH))]
        for i in range(NT - 1):
            block(lambda: _weave(grads[i][0], *([grads[i - 1][1]] if i else []),
                                 (pacer(accs[i], dyM, work),
                                  [f for c in range(4) for f in bwd_finish(i, c, accs[i])])))
            cp_dx[i].start()

        def grad_wo(i):
            def store(v, rows):
                dwo[0, rows] = dwo[0, rows] + v if i else v
                return probe(dwo, 0)
            return segments(lambda: _dot(wide(oT, 4 * i, 4), gb[i, 0:D], _NT), D, store)

        i = NT - 1
        block(lambda: _weave(grads[i][0] + [grad_wo(0)], grads[i - 1][1],
                             cut((pacer(accs[i], dyM, work),
                                  [f for c in range(4) for f in bwd_finish(i, c, accs[i])]), 0, 0.5)))
        cp_dwqkv[0].start()
        block(lambda: _weave([grad_wo(1), grad_wo(2)], grads[i][1],
                             cut((pacer(accs[i], dyM, work),
                                  [f for c in range(4) for f in bwd_finish(i, c, accs[i])]), 0.5, 1)))
        cp_dx[i].start()
        cp_dwqkv[1].start()
        _weave([grad_wo(3)])
        wo_b[...] = dwo[0, 0:D].astype(bf16)

        cp_dwo.start()

        db1 = [jnp.sum(db1_s[j], 0, keepdims=True) for j in range(NF)]
        db1_ref[...] = jnp.concatenate(db1, 1).astype(bf16)
        db2 = jnp.concatenate([db1_s[NF], db1_s[NF + 1, :, 0:L]], 1)
        db2_ref[...] = jnp.sum(db2, 0, keepdims=True)[:, 0:D].astype(bf16)

        for j in (NF - 2, NF - 1):
            for n in range(2):
                cp_dw(j, n).wait()
        for c in cp_out + cp_dx + cp_dwqkv + [cp_dwo]:
            c.wait()

    pl.run_scoped(epilogue, V((NT, D, TS), bf16), V((NT, D, TS), bf16), V((D, D), bf16), V((D, L), f32),
                  V((7, *_words(DH, QH)), u32), V((7, *_words(DH, NT * TH)), u32), V((7, *_words(QH, NT * TH)), u32),
                  V((2, D + 8, TH), f32), V((2, D + 8, L), f32), V((1, D + 8, D), f32),
                  *[V((7, DH + 8, TH), f32)] * (NT + 2))


@jax.jit
def pallas_parallel_sum__sliding_local_dilated__mixer_channel_mlp__prompt_kernel(
        A_x, A_wqkv, A_wo, B_x, B_w1, B_b1, B_w2, B_b2, grad_out):
    del B_x
    V = pltpu.VMEM
    hbm = pl.BlockSpec(memory_space=pl.ANY)
    vmem = pl.BlockSpec(memory_space=pltpu.VMEM)
    sds = lambda *s: jax.ShapeDtypeStruct(s, bf16)
    outT, dxT, dwqkv, dwo, dw1, db1, dw2T, db2 = pl.pallas_call(
        _kernel,
        in_specs=[hbm] * 6 + [vmem] * 2,
        out_specs=[hbm] * 5 + [vmem, hbm, vmem],
        out_shape=[sds(D, S), sds(D, S), sds(D, 3 * D), sds(D, D), sds(D, F), sds(1, F), sds(D, F), sds(1, D)],
        scratch_shapes=[
            V((NT, D + 16, TS), bf16), V((NT, D + 16, TS), bf16), V((1, D + 16, 3 * D), bf16), V((D, D), bf16),
            V((2 * RING, D + 16, FC), bf16), V((4, D, FC), bf16), V((4, STACK, L), f32), V((NT, 4, 1, TS), f32),
            V((NT, STACK, L), f32), V((NT, STACK, L), f32), V((NL + 2, *_words(4 * D + 16, L)), u32),
            V((NL, *_words(D, L)), u32), V((NL, *_words(3 * D + 16, L)), u32),
            V((NF + 2, 8, FC), f32), pltpu.SMEM((2,), jnp.int32),
            pltpu.SemaphoreType.DMA((2 * NT + 2,)), pltpu.SemaphoreType.DMA((2 * RING + 4,)),
            pltpu.SemaphoreType.DMA((2 * NT + 3,)),
        ],
        compiler_params=pltpu.CompilerParams(vmem_limit_bytes=127 * 2**20),
    )(A_x[0].T, grad_out[0].T, A_wqkv, A_wo, B_w1, B_w2.T, B_b1.reshape(1, F), B_b2.reshape(1, D))
    return (outT.T[None], dxT.T[None], dwqkv, dwo, dw1, db1.reshape(F), dw2T.T, db2.reshape(D))
```

```python
import jax
import jax.numpy as jnp
import jax.experimental.pallas as pl
import jax.experimental.pallas.tpu as pltpu

S, D, F = 2048, 576, 4608
H, HD, W, DIL = 32, 18, 8, 2
EPS = 1e-5
L = 128
TS, FC = 512, 512
TH, FH, DH, DQ = TS // 2, FC // 2, D // 2, D // 4
NT, NF, NL = S // TS, F // FC, S // L
RING = 4
QH = 896
STACK = 7168
DP = 640
bf16, f32, u32 = jnp.bfloat16, jnp.float32, jnp.uint32
_NN = (((1,), (0,)), ((), ()))
_NT = (((1,), (1,)), ((), ()))
C0 = 0.7978845608028654
C1 = 0.044715
KW = (256, 256, 384, 384, 256, 384, 384)


def _dot(a, b, dims=_NN):
    return jax.lax.dot_general(a, b, dims, preferred_element_type=f32)


def _words(rows, cols):
    return (rows // 2, cols)


def _ld(ref, idx=(), r0=0, n=None, cols=slice(None)):
    rows = slice(None) if n is None else pl.ds(r0 // 2, n // 2)
    return pltpu.bitcast(ref[(*idx, rows, cols)], bf16)


def _pack(v):
    n = v.shape[0] // 2
    return pltpu.bitcast(pltpu.pack_elementwise([v[:n], v[n:]], packed_dtype=bf16), u32)


def _unpack(w):
    w = pltpu.bitcast(w, u32)
    return jnp.concatenate([pltpu.bitcast(w << 16, f32), pltpu.bitcast(w & u32(0xFFFF0000), f32)], 0)


def _split(ref, idx, r0, n):
    return jnp.concatenate([ref[(*idx, pl.ds(r0 + e, n // 2, stride=2))] for e in range(2)], 0)


def _st(ref, idx, r0, v, c0=0):
    ref[(*idx, pl.ds(r0 // 2, v.shape[0] // 2), pl.ds(c0, v.shape[1]))] = _pack(v)


LEFT = ((1, 4), (3, 4), (1,), (4,), (1, 2), (3, -1), (2, -4))
RIGHT = ((1, 4), (1,), (2, -4), (3, -1), (4,), (1, 2), (3, 4))
OUT = ((1, 4, -5, 7), (3, 5), (2, 4), (1, -2, 3, 6))
LEFT_T = ((1, -4), (3, -4), (2, -4), (3, -1), (1, -2), (4,), (1,))
OUT_T = ((1, 6, -5, 3), (7, -5), (2, 6), (2, -1, 7, 4))


def _sum(terms, get):
    v = get(terms[0] - 1)
    for term in terms[1:]:
        v = v + get(term - 1) if term > 0 else v - get(-term - 1)
    return v


def _sums(scheme, xs):
    return [_sum(terms, lambda n: xs[n]) for terms in scheme]


def _sum2(scheme, outer, inner, get):
    return _sum(scheme[outer], lambda a: _sum(scheme[inner], lambda b: get(a, b)))


def _sums2(scheme, outer, get):
    return _sums(scheme, [_sum(scheme[outer], lambda a: get(a, b)) for b in range(4)])


_aset = lambda *x: _sums(LEFT, x)
_bset = lambda *x: _sums(RIGHT, x)
_tset = lambda *x: _sums(LEFT_T, x)
_post = lambda m: _sums(OUT, m)


def _weave(main, *sides):
    main = [f for item in main for f in (item if isinstance(item, list) else [item])]
    done = [0] * len(sides)
    if not main:
        return
    for n, item in enumerate(main):
        v = item()
        for s, (pace, side) in enumerate(sides):
            upto = (n + 1) * len(side) // len(main)
            if done[s] < upto and v is not None and pace is not None:
                pace(v())
            while done[s] < upto:
                side[done[s]]()
                done[s] += 1


def _kernel(xT_hbm, gT_hbm, wqkv_hbm, wo_hbm, w1_hbm, w2T_hbm, b1_ref, b2_ref,
            outT_hbm, dxT_hbm, dwqkv_hbm, dwo_hbm, dw1_hbm, db1_ref, dw2T_hbm, db2_ref,
            xb, gb, wqkv_b, wo_b, w_b, dw_b, acc_w, stats, outM, dyM, qkv, oT, dT, db1_s, zero_s, sem_in, sem_w, sem_out):

    def tile_in(src, dst, i, s):
        return pltpu.make_async_copy(src.at[:, pl.ds(i * TS, TS)], dst.at[i, pl.ds(0, D)], sem_in.at[s])

    cp_g = [tile_in(gT_hbm, gb, i, i) for i in range(NT)]
    cp_x = [tile_in(xT_hbm, xb, i, NT + i) for i in range(NT)]
    cp_wo = pltpu.make_async_copy(wo_hbm, wo_b, sem_in.at[2 * NT])
    cp_wqkv = pltpu.make_async_copy(wqkv_hbm, wqkv_b.at[0, pl.ds(0, D)], sem_in.at[2 * NT + 1])

    def cols(j):
        return pl.ds(j * FC if isinstance(j, int) else pl.multiple_of(j * FC, FC), FC)

    def cp_w(j, n):
        slot = n * RING + (j & RING - 1)
        return pltpu.make_async_copy((w1_hbm, w2T_hbm)[n].at[:, cols(j)], w_b.at[slot, pl.ds(0, D)], sem_w.at[slot])

    def cp_dw(j, n):
        slot = 2 * n + (j & 1)
        return pltpu.make_async_copy(dw_b.at[slot], (dw1_hbm, dw2T_hbm)[n].at[:, cols(j)], sem_w.at[2 * RING + slot])

    for c in (cp_wo, cp_g[0]):
        c.start()
    zero_s[0] = 0
    tie = {"z": zero_s[0]}

    def pacer(*refs, slab=0):
        def pace(v):
            for ref in refs:
                w = pltpu.bitcast(v, ref.dtype)
                rows = pl.ds(ref.shape[-2] - w.shape[0], w.shape[0])
                ref[(tie["z"] + slab,) + (0,) * (len(ref.shape) - 3) + (rows, slice(0, L))] = w
        return pace

    def probe(ref, first, r0=0):
        return lambda: ref[tie["z"] + first, pl.ds(r0, 8), pl.ds(0, L)]

    def fenced(main, sides, stops, gate, written):
        legs = [(lo, hi, free) for lo, (hi, free) in zip([0] + [f for _, f in stops], stops)]
        span, done = sum(hi - lo for lo, hi, _ in legs), 0
        for lo, hi, free in legs:
            _weave(main[lo:hi], *[cut(v, done / span, (done + hi - lo) / span) for v in sides])
            _weave(main[hi:free])
            done += hi - lo
            for src in written:
                m = 16 if src.dtype == bf16 else 8
                gate(src[tie["z"], pl.ds(pl.multiple_of(tie["z"], m), m), 0:L])
        _weave(main[stops[-1][1]:])

    def block(body):
        pl.when(tie["z"] == 0)(body)

    def segments(product, rows, store):
        n, held = rows // 4, {}

        def segment(r):
            def run():
                if r == 0:
                    held[0] = product()
                return store(held[0][n * r:n * (r + 1)], pl.ds(n * r, n))
            return run
        return [segment(r) for r in range(4)]

    def cut(stream, a, b):
        pace, todo = stream
        return pace, todo[int(len(todo) * a):int(len(todo) * b)]

    def aligned(v, m):
        return v if isinstance(v, int) else pl.multiple_of(v, m)

    def finish_dw(j, quarter):
        n, r0 = quarter >> 1, aligned((quarter & 1) * (DQ // 2), 8)
        acc = acc_w.at[0, pl.ds(aligned(STACK * (2 * (j & 1) + n), 1024), STACK)]

        def piece(r, b):
            def run():
                parts = [_sum(OUT[b], lambda m: acc[pl.ds(r0 + (DQ * (7 * k + m) + 8 * r), 8)]) for k in range(7)]
                for a, v in enumerate(_sums(OUT, parts)):
                    dw_b[2 * n + (j & 1), pl.ds(r0 + (DH * (a // 2) + DQ * (b // 2) + 8 * r), 8),
                         pl.ds(FH * (a % 2) + L * (b % 2), L)] = v.astype(bf16)
            return run
        return pacer(acc_w), [piece(r, b) for r in range(DQ // 16) for b in range(4)]

    def normed(x, i, c, twice):
        m1, r1, m2, r2 = [stats[i, n, :, pl.ds(L * c, L)] for n in range(4)]
        xn = (x - m1) * r1
        return (xn - m2) * r2 if twice else xn

    def main_phases(ya, ga, yTa, gTa, wB, b1_s):
        def right_w(j, quarter):
            n, r0 = quarter >> 1, aligned((quarter & 1) * L, L)
            src, dst = w_b.at[n * RING + (j & RING - 1)], wB.at[pl.ds(7 * (2 * (j & 1) + n), 7)]

            def piece(r):
                def run():
                    q = lambda a, c: _unpack(src[pl.ds(r0 + (256 * a + 16 * r), 16), c * FH:(c + 1) * FH])
                    for k, v in enumerate(_bset(q(0, 0), q(0, 1), q(1, 0), q(1, 1))):
                        dst[k, pl.ds(aligned(r0 >> 1, 8) + 8 * r, 8)] = _pack(v)
                return run

            def tail():
                for k, c in ((2, 1), (3, 0), (5, 1), (6, 0)):
                    dst[k, 128:160] = pltpu.bitcast(src[512:576, c * FH:(c + 1) * FH], u32)
                    rows = jax.lax.broadcasted_iota(jnp.int32, (16, FH), 0)
                    b = jnp.broadcast_to(b1_s[j, :, c * FH:(c + 1) * FH], (16, FH))
                    dst[k, 160:168] = _pack(jnp.where(rows < 1 - n, b, 0.0))
            return pacer(w_b), [piece(r) for r in range(L // 16)] + [tail]

        def source(is_x, twice):
            def get(i, r0, n, c, unpack=_unpack):
                v = unpack((xb if is_x else gb)[i, pl.ds(r0, n), pl.ds(L * c, L)])
                return normed(v, i, c, twice) if is_x else v
            return get

        def combos_T(get, dst, i, r):
            st = {}

            def load():
                for a in range(4):
                    for b in range(4):
                        st[a, b] = get(i, DH * (a // 2) + DQ * (b // 2) + 16 * r, 16, 2 * (a % 2) + b % 2)

            def sums(k):
                def run():
                    for n, v in enumerate(_sums2(LEFT, k, lambda a, b: st[a, b])):
                        _st(dst, (0,), STACK * i + DQ * (7 * k + n) + 16 * r, v)
                return run
            return [load] + [sums(k) for k in range(7)]

        def prologue(wP, xB, nat):
            def norm(i, c):
                cs = pl.ds(L * c, L)
                stat = lambda n: stats[i, n, :, cs]
                terms = (lambda x: x, lambda x: jnp.square(x - stat(0)), lambda x: (x - stat(0)) * stat(1),
                         lambda x: jnp.square((x - stat(0)) * stat(1) - stat(2)))

                def sweep(n):
                    def run():
                        total = 0.0
                        for r in range(0, D, 64):
                            v = terms[n](_unpack(xb[i, pl.ds(r, 64), cs]))
                            total = total + sum(v[8 * m:8 * m + 8] for m in range(1, 8)) + v[0:8]
                        mean = jnp.sum(total, 0, keepdims=True) * (1.0 / D)
                        stats[i, n, :, cs] = jax.lax.rsqrt(mean + EPS) if n % 2 else mean
                    return run
                return [sweep(n) for n in range(4)]

            def flip(get, i, c, r, fill):
                def run():
                    n = min(L, D - L * r)
                    v = get(i, L * r, n, c, lambda w: w.astype(f32))
                    if n < L:
                        row = jax.lax.broadcasted_iota(jnp.int32, (L - n, L), 0)
                        v = jnp.concatenate([v, jnp.where(row == 0, fill, 0.0)], 0)
                    nat[r, pl.ds(L * c, L)] = v.T
                return run

            def wide_aset(q):
                blocks = (q(0, 0, 2), q(0, 2, 2), q(1, 0, 2), q(1, 2, 2))
                t1, t2 = q(0, 4, 1), q(1, 4, 1)
                tails = {2: t1, 3: t2, 5: t2 - t1, 6: t1 - t2}
                return [jnp.concatenate([v, tails[k]], 1) if k in tails else v
                        for k, v in enumerate(_aset(*blocks))], blocks, t1 + t2

            def combos_N(dst, i, r, is_g):
                def run():
                    q = lambda half, c0, n: jnp.concatenate(
                        [_split(nat, (c0 + u,), TH * half + 16 * r, 16) for u in range(n)], 1)
                    vs, blocks, tail = wide_aset(q)
                    for k, v in enumerate(vs):
                        _st(dst, (7 * i + k,), 16 * r, v)
                    if is_g:
                        t = jnp.concatenate([blocks[0] + blocks[2], blocks[1] + blocks[3], tail], 1)
                        t = t[0:8] + t[8:16]
                        db1_s[NF] += t[:, 0:FC]
                        db1_s[NF + 1, :, 0:L] += t[:, FC:DP]
                return run

            def layouts(i, is_x):
                get = source(is_x, True)
                return ([flip(get, i, c, r, 1.0 if is_x else 0.0) for c in range(4) for r in range(5)] +
                        [f for r in range(DQ // 16 if is_x else 0) for f in combos_T(get, yTa, i, r)] +
                        [combos_N(ya if is_x else ga, i, r, not is_x) for r in range(TH // 16)])

            def right(i):
                def piece(r, c):
                    return lambda: _st(xB, (i % 2,), 64 * r, source(True, False)(i, 64 * r, 64, c), L * c)
                return [piece(r, c) for r in range(D // 64) for c in range(4)]

            def put_left(part, r, v):
                for e in range(2):
                    wP[part, pl.ds(DH * e + 16 * r, 16), :] = v[16 * e:16 * (e + 1), 0:D].astype(bf16)

            def flip_w(c, r):
                def run():
                    n, m = min(L, 3 * D - L * c), min(L, D - L * r)
                    v = wqkv_b[0, pl.ds(L * r, m), pl.ds(L * c, n)].astype(f32)
                    if n < L:
                        v = jnp.concatenate([v, jnp.zeros((m, L - n), f32)], 1)
                    if m < L:
                        v = jnp.concatenate([v, jnp.zeros((L - m, L), f32)], 0)
                    nat[r, pl.ds(TS + L * c, L)] = v.T
                return run

            def left_w(part):
                def piece(r):
                    return lambda: put_left(part, r, jnp.concatenate(
                        [_split(nat, (u,), TS + D * part + 32 * r, 32) for u in range(5)], 1))
                return [piece(r) for r in range(D // 32)]

            def project(i, part):
                def item(c, e):
                    rows, cs, n = pl.ds(DQ * e, DQ), pl.ds(TH * c, TH), DQ // 3

                    def segment(r, held):
                        def run():
                            if r == 0:
                                rhs = gb[i, 0:D, cs] if part == 3 else _ld(xB, (i % 2,), cols=cs)
                                held.append(_dot(jnp.concatenate(
                                    [wP[part, pl.ds(DH * u + DQ * e, DQ), :] for u in range(2)], 0), rhs))
                            v = jnp.concatenate([held[0][DQ * u + n * r:DQ * u + n * (r + 1)] for u in range(2)], 0)
                            at = DH * part + DQ * e + n * r
                            for u in range(2):
                                qkv[4 * i + 2 * c + u + 1, pl.ds(at, n)] = _pack(v[:, L * u:L * (u + 1)])
                            return probe(qkv, 4 * i + 2 * c + 1, at)
                        return run
                    held = []
                    return [segment(r, held) for r in range(3)]
                return [item(c, e) for c in range(2) for e in range(2)]

            def setup():
                b = b1_ref[...].astype(f32).reshape(1, F)
                for j in range(NF):
                    b1_s[j] = b[:, FC * j:FC * (j + 1)]
                for k in range(28):
                    wB[k, 160:192, :] = jnp.zeros((32, FH), u32)
                db1_s[...] = jnp.zeros(db1_s.shape, f32)
                for t in (0, NL + 1):
                    qkv[t] = jnp.zeros(qkv.shape[1:], u32)

            later = [cp_g[1], cp_wqkv, cp_x[0], cp_g[2], cp_g[3], cp_x[1], cp_x[2], cp_x[3]]
            later += [cp_w(j, n) for j in range(3) for n in range(2)]
            for c in later[:3]:
                c.start()
            setup()
            cp_wo.wait()
            for r in range(D // 32):
                put_left(3, r, _unpack(wo_b[pl.ds(32 * r, 32), :]))
            cp_g[0].wait()
            pg, px, pw = pacer(gb), pacer(xb), pacer(nat)

            flips = [flip_w(c, r) for c in range(14) for r in range(5)]

            def job(i, part):
                stats_of = lambda m: (px, [f for c in range(4) for f in norm(m, c)] + right(m))
                if part == 3:
                    sides = ([(pg, layouts(0, False))], [(pw, flips[:35])], [(pw, flips[35:])],
                             [stats_of(0), (pw, left_w(0))])[i]
                else:
                    sides = [(pw, left_w(part + 1))] if i == 0 and part < 2 else []
                    if part == 0 and i > 0:
                        sides.append((pg, layouts(i, False)))
                    if part > 0:
                        todo = layouts(i, True)
                        sides.append((px, todo[:20] + todo[-16:] if part == 1 else todo[20:-16]))
                    if part == 2:
                        sides += [stats_of(i + 1)] if i + 1 < NT else [right_w(0, m) for m in range(4)]
                _weave(project(i, part), *sides)

            for i in range(NT):
                for c in later[3 + 2 * i:5 + 2 * i]:
                    c.start()
                (cp_g[i + 1] if i + 1 < NT else cp_x[0]).wait()
                if i == 1:
                    cp_wqkv.wait()
                block(lambda: job(i, 3))
            for c in later[11:]:
                c.start()
            for i in range(NT):
                for part in range(3):
                    if part == 2:
                        for c in [cp_x[i + 1]] if i + 1 < NT else later[8:12]:
                            c.wait()
                    block(lambda: job(i, part))

        pl.run_scoped(prologue,
                      pltpu.VMEM((4, D, D), bf16), pltpu.VMEM((2, *_words(D, TS)), u32),
                      pltpu.VMEM((5, TS + 14 * L + 8, L), f32))

        def mlp(wA, mp, md, hB, dB, p_s, dl_s, hd_s):
            tie["z"] = zero_s[0]

            def left_w(j, quarter):
                n, r0 = quarter >> 1, aligned((quarter & 1) * 64, 64)
                src, dst = w_b.at[n * RING + (j & RING - 1)], wA.at[0, pl.ds(aligned(STACK // 2 * (2 * (j & 1) + n), 512), STACK // 2)]

                def piece(r, k):
                    def run():
                        q = lambda a, b: _unpack(src[pl.ds(r0 + (DH * (a // 2) + DQ * (b // 2) + 16 * r), 16),
                                                     pl.ds(FH * (a % 2) + L * (b % 2), L)])
                        for m, v in enumerate(_sums2(LEFT_T, k, q)):
                            dst[pl.ds(aligned(r0 >> 1, 8) + (DQ // 2 * (7 * k + m) + 8 * r), 8)] = _pack(v)
                    return run
                return pacer(w_b), [piece(r, k) for r in range(5) for k in range(7)]

            def stage_A(n):
                i, j = n & 3, n >> 2

                def item(xa, w, m, k):
                    def store(v, rows):
                        m[2 * k, rows] = v[:, 0:L]
                        m[2 * k + 1, rows] = v[:, L:FH]
                        return probe(m, 2 * k)
                    return segments(lambda: _dot(_ld(xa, (7 * i + k,), cols=slice(0, KW[k])),
                                                 _ld(wB, (7 * (2 * (j & 1) + w) + k,), 0, KW[k])), TH, store)
                return [item(ya, 0, mp, k) for k in range(7)] + [item(ga, 1, md, k) for k in range(7)]

            def stage_G(n):
                def piece(r, c):
                    st = {}

                    def total(m, e):
                        return _post([m[2 * k + c, pl.ds(16 * r + e, 8, stride=2)] for k in range(7)])

                    def act(e):
                        def run():
                            st["h", e], st["g"] = [], []
                            for p in total(mp, e):
                                p2 = p * p
                                a = 0.5 + 0.5 * jnp.tanh(p * (C0 + (C0 * C1) * p2))
                                h = p * a
                                st["h", e].append(h)
                                st["g"].append(a + (h - h * a) * (2 * C0 + (6 * C0 * C1) * p2))
                            if e == 1:
                                emit(hB, "h")
                        return run

                    def grad(e):
                        def run():
                            st["d", e] = [d * g for d, g in zip(total(md, e), st["g"])]
                            if e == 1:
                                emit(dB, "d")
                                for half in range(2):
                                    t = (st["d", 0][half] + st["d", 0][2 + half]) + (st["d", 1][half] + st["d", 1][2 + half])
                                    where = pl.ds(half * FH + L * c, L)
                                    db1_s[n >> 2, :, where] += t
                        return run

                    def emit(dst, name):
                        for q, v in enumerate(zip(st[name, 0], st[name, 1])):
                            at = (r % 8, "hd".index(name), 2 * (r // 8) + c, q)
                            hd_s[at] = jnp.concatenate(v, 0)
                    return [act(0), grad(0), act(1), grad(1)]

                def second(r, w, k):
                    def run():
                        for m, v in enumerate(_sums2(RIGHT, k, lambda a, b: hd_s[r, w, b, a])):
                            _st((hB, dB)[w], (7 * k + m,), 16 * r, v)
                    return run
                return ((pacer(mp, md),
                         [f for r in range(TH // 16) for c in range(2) for f in piece(r, c)]),
                        (pacer(hd_s, slab=8), [second(r, w, k) for w in range(2) for r in range(L // 16) for k in range(7)]))

            def stage_BC(n):
                i, j = n & 3, n >> 2
                plan = (((acc_w, 2 * (j & 1) + 1), i > 0, (gTa, i), hB, _NN),
                        ((acc_w, 2 * (j & 1)), i > 0, (yTa, i), dB, _NN),
                        ((outM, i), j > 0, (wA, 2 * (j & 1) + 1), hB, _NT),
                        ((dyM, i), j > 0, (wA, 2 * (j & 1)), dB, _NT))
                jobs = [(*p, k) for p in plan for k in range(49)]

                def group(four):
                    m, held = DQ // 3, []

                    def segment(r):
                        def run():
                            if r == 0:
                                held.extend(_dot(pltpu.bitcast(a[0, pl.ds(aligned(STACK // 2 * at, 512) + DQ // 2 * k, DQ // 2)], bf16), _ld(b, (k,), 0, L), dims)
                                            for _, _, (a, at), b, dims, k in four)
                            old = [jnp.where(started, acc[0, pl.ds(aligned(STACK * at, 1024) + (DQ * k + m * r), m)], 0.0)
                                   for (acc, at), started, *_, k in four]
                            for ((acc, at), *_, k), u, v in zip(four, old, held):
                                acc[0, pl.ds(aligned(STACK * at, 1024) + (DQ * k + m * r), m)] = u + v[m * r:m * (r + 1)]
                            return probe(acc, 0, aligned(STACK * at, 1024) + DQ * k)
                        return run
                    return [segment(r) for r in range(3)]
                return [group(jobs[k:k + 4]) for k in range(0, len(jobs), 4)]

            def attention(t, hg):
                st = {}
                lane = lambda: jax.lax.broadcasted_iota(jnp.int32, (8, L), 1)

                def rows(part, d):
                    return pl.ds((part * D + 8 * HD * hg) // 2 + d, 8, stride=HD // 2)

                def ld(dt, part, d):
                    return qkv[t + 1 + dt, rows(part, d), :]

                def back(cur, prev, w):
                    if w == 0:
                        return cur
                    return pltpu.roll(jnp.where(lane() < L - DIL * w, cur, prev), DIL * w, 1)

                def ahead(cur, nxt, w):
                    if w == 0:
                        return cur
                    return pltpu.roll(jnp.where(lane() >= DIL * w, cur, nxt), L - DIL * w, 1)

                def scores(own, other, dst, d):
                    def run():
                        a, cur, prev = _unpack(ld(0, own, d)), ld(0, other, d), ld(-1, other, d)
                        for w in range(W):
                            v = a * _unpack(back(cur, prev, w))
                            v = v[0:8] + v[8:16]
                            st[w] = v if d == 0 else st[w] + v
                            if d == HD // 2 - 1:
                                dst[t & 3, hg, w] = st[w]
                    return run

                def soft():
                    pos = lane() + t * L
                    lg = [jnp.where(pos >= DIL * w, p_s[t & 3, hg, w] * HD ** -0.5, -1e9) for w in range(W)]
                    m = lg[0]
                    for w in range(1, W):
                        m = jnp.maximum(m, lg[w])
                    e = [jnp.exp(x - m) for x in lg]
                    tot = e[0]
                    for w in range(1, W):
                        tot = tot + e[w]
                    inv = 1.0 / tot
                    p = [x * inv for x in e]
                    dp = [dl_s[t & 3, hg, w] for w in range(W)]
                    c = p[0] * dp[0]
                    for w in range(1, W):
                        c = c + p[w] * dp[w]
                    for w in range(W):
                        p_s[t & 3, hg, w] = p[w]
                        dl_s[t & 3, hg, w] = jnp.where(pos >= DIL * w, p[w] * (dp[w] - c) * HD ** -0.5, 0.0)

                def gather(src, other, dst, part, d):
                    def run():
                        if d == 0:
                            for w in range(W):
                                st[w] = jnp.concatenate([src[t & 3, hg, w]] * 2, 0)
                        cur, prev = ld(0, other, d), ld(-1, other, d)
                        v = st[0] * _unpack(cur)
                        for w in range(1, W):
                            v = v + st[w] * _unpack(back(cur, prev, w))
                        dst[t, rows(part, d), :] = _pack(v)
                    return run

                def scatter(src, other, dst, part, d):
                    def run():
                        if d == 0:
                            for w in range(W):
                                st[w] = jnp.concatenate([ahead(src[t & 3, hg, w], src[(t + 1) & 3, hg, w], w)] * 2, 0)
                        cur, nxt = ld(0, other, d), ld(1, other, d)
                        v = st[0] * _unpack(cur)
                        for w in range(1, W):
                            v = v + st[w] * _unpack(ahead(cur, nxt, w))
                        dst[t, rows(part, d), :] = _pack(v)
                    return run

                ds = range(HD // 2)
                return ([scores(0, 1, p_s, d) for d in ds] + [scores(3, 2, dl_s, d) for d in ds] + [soft] +
                        [gather(p_s, 2, oT, 0, d) for d in ds] + [gather(dl_s, 1, dT, 0, d) for d in ds] +
                        [scatter(dl_s, 0, dT, 1, d) for d in ds] + [scatter(p_s, 3, dT, 2, d) for d in ds])

            for ref in (p_s, dl_s):
                ref[0] = jnp.zeros(ref.shape[1:], f32)

            def wipe(k):
                def run():
                    acc_w[0, pl.ds(STACK * (2 + k // 49) + DQ * (k % 49), DQ)] = jnp.zeros((DQ, L), f32)
                return run
            rows_g = lambda tiles: (pacer(gb), [f for i in tiles for r in range(DQ // 16)
                                                for f in combos_T(source(False, False), gTa, i, r)])
            block(lambda: _weave(stage_A(0), *[left_w(0, m) for m in range(4)], rows_g((0, 1))))

            block(lambda: _weave(stage_G(0)[0][1], (None, rows_g((2,))[1])))
            block(lambda: _weave(stage_A(1), stage_G(0)[1], right_w(1, 0), rows_g((3,)),
                                 (pacer(hB), [wipe(k) for k in range(98)])))

            def step(n, carry):
                tie["z"] = zero_s[0]
                i, j = n & 3, n >> 2

                @pl.when(i == NT - 1)
                def _():
                    for w in range(2):
                        pl.when(j >= 2)(lambda: cp_dw(j - 2, w).wait())
                        pl.when(j + 2 < NF)(lambda: cp_w(j + 2, w).wait())
                        pl.when(j + 3 < NF)(lambda: cp_w(j + 3, w).start())

                @pl.when((i == 0) & (j >= 2))
                def _():
                    for w in range(2):
                        cp_dw(j - 2, w).start()

                m = jnp.minimum(n, 2 * NL - 2 + (n & 1))
                att = (pacer(qkv), [f for u in range(2) for f in attention(NL - 1 - (m >> 1), 2 * (m & 1) + u)])
                g, x = stage_G(n + 1), 0.9
                main = stage_BC(n)
                _weave(main[:-1], g[0], cut(att, 0, x),
                       right_w(jnp.minimum(((n + 1) >> 2) + 1, NF - 1), (n + 1) & 3))
                _weave(main[-1:])
                sides = [g[1], cut(att, x, 1), left_w(jnp.minimum(j + 1, NF - 1), i), finish_dw(j + 1, i)]
                fenced(stage_A(n + 2), sides, ((5, 7), (10, 12)), pacer(ga, slab=NT * 7), (oT, dT, wA, hB, dB, dw_b))
                return carry

            jax.lax.fori_loop(0, NT * NF - 2, step, 0)
            tie["z"] = zero_s[0]


            def drain():
                n = NT * NF - 2
                main, g = stage_BC(n), stage_G(n + 1)
                _weave(main[:40], g[0], finish_dw(NF - 2, 2))
                _weave(main[40:])
                for f in cut(g[1], 0, 0.5)[1]:
                    f()
                main = stage_BC(n + 1)
                _weave(main[:10], cut(g[1], 0.5, 1))
                _weave(main[10:], finish_dw(NF - 2, 3))
            block(drain)
            for w in range(2):
                cp_dw(NF - 3, w).wait()
                cp_dw(NF - 2, w).start()

        V = pltpu.VMEM
        pl.run_scoped(
            mlp, V((1, *_words(4 * STACK, L)), u32), V((14, TH + 8, L), f32), V((14, TH + 8, L), f32),
            V((49, *_words(L + 16, L)), u32), V((49, *_words(L, L)), u32),
            V((4, 4, W, 8, L), f32), V((4, 4, W, 8, L), f32), V((9, 2, 4, 4, 16, L), f32))

    V = pltpu.VMEM
    pl.run_scoped(
        main_phases,
        V((NT * 7 + 1, *_words(TH, 384)), u32), V((NT * 7 + 1, *_words(TH, 384)), u32),
        V((1, *_words(NT * STACK, L)), u32), V((1, *_words(NT * STACK, L)), u32),
        V((4 * 7, *_words(384, FH)), u32), V((NF, 1, FC), f32))

    def epilogue(out_b, dx_b, woT, b2c, wT, xA, dS, fin, work, dwo, *accs):
        tie["z"] = zero_s[0]

        def tile_out(src, dst, i, s):
            return pltpu.make_async_copy(src.at[i], dst.at[:, pl.ds(i * TS, TS)], sem_out.at[s])

        cp_out = [tile_out(out_b, outT_hbm, i, i) for i in range(NT)]
        cp_dx = [tile_out(dx_b, dxT_hbm, i, NT + i) for i in range(NT)]
        cp_dwqkv = [pltpu.make_async_copy(wqkv_b.at[0, pl.ds(0, D), pl.ds(c, n)], dwqkv_hbm.at[:, pl.ds(c, n)],
                                          sem_out.at[2 * NT + 1 + m])
                    for m, (c, n) in enumerate(((0, 3 * TH), (3 * TH, 3 * D - 3 * TH)))]
        cp_dwo = pltpu.make_async_copy(wo_b, dwo_hbm, sem_out.at[2 * NT])

        def wide(ref, t, tiles, r0=0, n=None):
            return jnp.concatenate([_ld(ref, (t + u,), r0, n) for u in range(tiles)], 1)

        def flip_wo(c):
            n = min(L, D - L * c)
            v = wo_b[:, pl.ds(L * c, n)].astype(f32)
            b = b2_ref[...].astype(f32).reshape(1, D)[:, L * c:L * c + n]
            if n < L:
                v = jnp.concatenate([v, jnp.zeros((D, L - n), f32)], 1)
                b = jnp.concatenate([b, jnp.zeros((1, L - n), f32)], 1)
            v = jnp.concatenate([v, jnp.zeros((DP - D, L), f32)], 0)
            woT[pl.ds(L * c, n), :] = v.T[0:n, 0:D].astype(bf16)
            b2c[pl.ds(L * c, n), :] = jnp.broadcast_to(b, (L, L)).T[0:n]

        def left_w(r):
            def run():
                def q(half, c):
                    w = min(QH, 3 * D - QH * c)
                    v = _unpack(wqkv_b[0, pl.ds(DH * half + 16 * r, 16), pl.ds(QH * c, w)])
                    return v if w == QH else jnp.concatenate([v, jnp.zeros((16, QH - w), f32)], 1)
                for k, v in enumerate(_tset(q(0, 0), q(0, 1), q(1, 0), q(1, 1))):
                    _st(wT, (k,), 16 * r, v)
            return run

        def left_x(i, r, u):
            def run():
                q = lambda r0, c: normed(_unpack(xb[i, pl.ds(r0 + 48 * r, 48), pl.ds(L * (2 * c + u), L)]),
                                         i, 2 * c + u, False)
                for k, v in enumerate(_aset(q(0, 0), q(0, 1), q(DH, 0), q(DH, 1))):
                    _st(xA, (k,), 48 * r, v, TH * i + L * u)
            return run

        def right_d(i, r, u):
            def run():
                def q(half, c):
                    if QH * half + 32 * r >= 3 * D:
                        return jnp.zeros((32, L), f32)
                    return _unpack(dT[4 * i + 2 * c + u, pl.ds((QH * half + 32 * r) // 2, 16)])
                for k, v in enumerate(_bset(q(0, 0), q(1, 0), q(0, 1), q(1, 1))):
                    _st(dS, (k,), 32 * r, v, TH * i + L * u)
            return run

        def rights(i):
            return [right_d(i, r, u) for r in range(QH // 32) for u in range(2)]

        def fwd(i, half, a):
            def store(v, rows):
                fin[half, pl.ds(DH * a + rows.start, rows.size)] = v
                return probe(fin, half)
            return segments(lambda: _dot(woT[pl.ds(DH * a, DH), :], wide(oT, 4 * i + 2 * half, 2)), DH, store)

        def fwd_finish(i, r, b):
            def run():
                parts = [_sum(OUT_T[b], lambda n: outM[0, pl.ds(STACK * i + DQ * (7 * k + n) + 8 * r, 8)]) for k in range(7)]
                for a, v in enumerate(_sums(OUT_T, parts)):
                    rows = pl.ds(DH * (a // 2) + DQ * (b // 2) + 8 * r, 8)
                    cs = pl.ds(TH * (a % 2) + L * (b % 2), L)
                    v = v + fin[a % 2, rows, pl.ds(L * (b % 2), L)] + b2c[rows, :] + xb[i, rows, cs].astype(f32)
                    out_b[i, rows, cs] = v.astype(bf16)
            return run

        def bwd(i, acc):
            def item(k):
                def store(v, rows):
                    acc[k, rows] = v
                    return probe(acc, k)
                return segments(lambda: _dot(_ld(wT, (k,)), _ld(dS, (k,), cols=pl.ds(TH * i, TH))), DH, store)
            return [item(k) for k in range(7)]

        def bwd_finish(i, c, acc):
            cs, st, n = pl.ds(L * c, L), {}, 48
            x = lambda r, twice: normed(xb[i, pl.ds(n * r, n), cs].astype(f32), i, c, twice)
            fold = lambda v: sum(v[8 * m:8 * m + 8] for m in range(1, n // 8)) + v[0:8]
            mean = lambda v: jnp.sum(v, 0, keepdims=True) * (1.0 / D)

            def tally(r, name, d, xn):
                work[c % 2, pl.ds(n * r, n)] = d
                s1, s2 = fold(d), fold(d * xn)
                st[name] = (s1, s2) if r == 0 else (st[name][0] + s1, st[name][1] + s2)
                if n * (r + 1) == D:
                    st[name] = [mean(v) for v in st[name]]

            def first(r):
                a, b, r0 = n * r // DH, n * r % DH // DQ, n * r % DQ
                dy = _sum2(OUT_T, 2 * a + c // 2, 2 * b + c % 2, lambda k, m: dyM[0, pl.ds(STACK * i + DQ * (7 * k + m) + r0, n)])
                tally(r, "y", dy, x(r, True))

            def second(r):
                dy, rs = work[c % 2, pl.ds(n * r, n)], pl.ds(n * r % DH, n)
                d = stats[i, 3, :, cs] * (dy - st["y"][0] - x(r, True) * st["y"][1])
                d = d + _sum(OUT_T[2 * (n * r // DH) + c // 2], lambda k: acc[k, rs, pl.ds(L * (c % 2), L)])
                tally(r, "x", d, x(r, False))

            def third(r):
                rs = pl.ds(n * r, n)
                d = stats[i, 1, :, cs] * (work[c % 2, rs] - st["x"][0] - x(r, False) * st["x"][1])
                dx_b[i, rs, cs] = (d + gb[i, rs, cs].astype(f32)).astype(bf16)
            return [lambda f=f, r=r: f(r) for f in (first, second, third) for r in range(D // n)]

        def grad_w(c, n, acc):
            def item(k):
                def store(v, rows):
                    acc[k, rows, 0:n] = v
                    return probe(acc, k)
                return segments(lambda: _dot(_ld(xA, (k,)), _ld(dS, (k,), c, n), _NT), DH, store)

            def finish(r, u):
                def run():
                    for q, v in enumerate(_post([acc[k, pl.ds(16 * r, 16), pl.ds(u, L)] for k in range(7)])):
                        c0 = QH * (q % 2) + c + u
                        w = min(L, 3 * D - c0)
                        wqkv_b[0, pl.ds(DH * (q // 2) + 16 * r, 16), pl.ds(c0, w)] = v[:, 0:w].astype(bf16)
                return run
            return [item(k) for k in range(7)], (pacer(acc), [finish(r, u) for r in range(18) for u in range(0, n, L)])

        for c in range(5):
            flip_wo(c)
        def tile(i):
            _weave([fwd(i, half, a) for half in range(2) for a in range(2)],
                   (pacer(xb), [left_x(i, r, u) for r in range(6) for u in range(2)]), finish_dw(NF - 1, i),
                   (None, [] if i else [left_w(r) for r in range(DH // 16)] + rights(0)))
            _weave(bwd(i, accs[i]), (pacer(dT), rights(i + 1) if i + 1 < NT else []),
                   (pacer(fin, outM), [fwd_finish(i, r, b) for r in range(DQ // 8) for b in range(4)]))

        for i in range(NT):
            block(lambda: tile(i))
            cp_out[i].start()
        for w in range(2):
            cp_dw(NF - 1, w).start()
        grads = [grad_w(c, min(TH, QH - c), accs[NT + n % 2]) for n, c in enumerate(range(0, QH, TH))]
        for i in range(NT - 1):
            block(lambda: _weave(grads[i][0], *([grads[i - 1][1]] if i else []),
                                 (pacer(accs[i], dyM, work),
                                  [f for c in range(4) for f in bwd_finish(i, c, accs[i])])))
            cp_dx[i].start()

        def grad_wo(i):
            def store(v, rows):
                dwo[0, rows] = dwo[0, rows] + v if i else v
                return probe(dwo, 0)
            return segments(lambda: _dot(wide(oT, 4 * i, 4), gb[i, 0:D], _NT), D, store)

        i = NT - 1
        block(lambda: _weave(grads[i][0] + [grad_wo(0)], grads[i - 1][1],
                             cut((pacer(accs[i], dyM, work),
                                  [f for c in range(4) for f in bwd_finish(i, c, accs[i])]), 0, 0.5)))
        cp_dwqkv[0].start()
        block(lambda: _weave([grad_wo(1), grad_wo(2)], grads[i][1],
                             cut((pacer(accs[i], dyM, work),
                                  [f for c in range(4) for f in bwd_finish(i, c, accs[i])]), 0.5, 1)))
        cp_dx[i].start()
        cp_dwqkv[1].start()
        _weave([grad_wo(3)])
        wo_b[...] = dwo[0, 0:D].astype(bf16)

        cp_dwo.start()

        db1 = [jnp.sum(db1_s[j], 0, keepdims=True) for j in range(NF)]
        db1_ref[...] = jnp.concatenate(db1, 1).astype(bf16).reshape(F)
        db2 = jnp.concatenate([db1_s[NF], db1_s[NF + 1, :, 0:L]], 1)
        db2_ref[...] = jnp.sum(db2, 0, keepdims=True)[:, 0:D].reshape(D).astype(bf16)

        for j in (NF - 2, NF - 1):
            for n in range(2):
                cp_dw(j, n).wait()
        for c in cp_out + cp_dx + cp_dwqkv + [cp_dwo]:
            c.wait()

    pl.run_scoped(epilogue, V((NT, D, TS), bf16), V((NT, D, TS), bf16), V((D, D), bf16), V((D, L), f32),
                  V((7, *_words(DH, QH)), u32), V((7, *_words(DH, NT * TH)), u32), V((7, *_words(QH, NT * TH)), u32),
                  V((2, D + 8, TH), f32), V((2, D + 8, L), f32), V((1, D + 8, D), f32),
                  *[V((7, DH + 8, TH), f32)] * (NT + 2))


@jax.jit
def pallas_parallel_sum__sliding_local_dilated__mixer_channel_mlp__prompt_kernel(
        A_x, A_wqkv, A_wo, B_x, B_w1, B_b1, B_w2, B_b2, grad_out):
    del B_x
    V = pltpu.VMEM
    hbm = pl.BlockSpec(memory_space=pl.ANY)
    vmem = pl.BlockSpec(memory_space=pltpu.VMEM)
    sds = lambda *s: jax.ShapeDtypeStruct(s, bf16)
    outT, dxT, dwqkv, dwo, dw1, db1, dw2T, db2 = pl.pallas_call(
        _kernel,
        in_specs=[hbm] * 6 + [vmem] * 2,
        out_specs=[hbm] * 5 + [vmem, hbm, vmem],
        out_shape=[sds(D, S), sds(D, S), sds(D, 3 * D), sds(D, D), sds(D, F), sds(F), sds(D, F), sds(D)],
        scratch_shapes=[
            V((NT, D + 16, TS), bf16), V((NT, D + 16, TS), bf16), V((1, D + 16, 3 * D), bf16), V((D, D), bf16),
            V((2 * RING, D + 16, FC), bf16), V((4, D, FC), bf16), V((1, 4 * STACK, L), f32), V((NT, 4, 1, TS), f32),
            V((1, NT * STACK, L), f32), V((1, NT * STACK, L), f32), V((NL + 2, *_words(4 * D + 16, L)), u32),
            V((NL, *_words(D, L)), u32), V((NL, *_words(3 * D + 16, L)), u32),
            V((NF + 2, 8, FC), f32), pltpu.SMEM((2,), jnp.int32),
            pltpu.SemaphoreType.DMA((2 * NT + 2,)), pltpu.SemaphoreType.DMA((2 * RING + 4,)),
            pltpu.SemaphoreType.DMA((2 * NT + 3,)),
        ],
        compiler_params=pltpu.CompilerParams(vmem_limit_bytes=127 * 2**20),
    )(A_x[0].T, grad_out[0].T, A_wqkv, A_wo, B_w1, B_w2.T, B_b1, B_b2)
    return (outT.T[None], dxT.T[None], dwqkv, dwo, dw1, db1, dw2T.T, db2)
```

```python
import jax
import jax.numpy as jnp
import jax.experimental.pallas as pl
import jax.experimental.pallas.tpu as pltpu

S, D, F = 2048, 576, 4608
H, HD, W, DIL = 32, 18, 8, 2
EPS = 1e-5
L = 128
TS, FC = 512, 512
TH, FH, DH, DQ = TS // 2, FC // 2, D // 2, D // 4
NT, NF, NL = S // TS, F // FC, S // L
RING = 4
QH = 896
STACK = 7168
DP = 640
bf16, f32, u32 = jnp.bfloat16, jnp.float32, jnp.uint32
_NN = (((1,), (0,)), ((), ()))
_NT = (((1,), (1,)), ((), ()))
C0 = 0.7978845608028654
C1 = 0.044715
KW = (256, 256, 384, 384, 256, 384, 384)


def _dot(a, b, dims=_NN):
    return jax.lax.dot_general(a, b, dims, preferred_element_type=f32)


def _words(rows, cols):
    return (rows // 2, cols)


def _ld(ref, idx=(), r0=0, n=None, cols=slice(None)):
    rows = slice(None) if n is None else pl.ds(r0 // 2, n // 2)
    return pltpu.bitcast(ref[(*idx, rows, cols)], bf16)


def _pack(v):
    n = v.shape[0] // 2
    return pltpu.bitcast(pltpu.pack_elementwise([v[:n], v[n:]], packed_dtype=bf16), u32)


def _unpack(w):
    w = pltpu.bitcast(w, u32)
    return jnp.concatenate([pltpu.bitcast(w << 16, f32), pltpu.bitcast(w & u32(0xFFFF0000), f32)], 0)


def _split(ref, idx, r0, n):
    return jnp.concatenate([ref[(*idx, pl.ds(r0 + e, n // 2, stride=2))] for e in range(2)], 0)


def _st(ref, idx, r0, v, c0=0):
    ref[(*idx, pl.ds(r0 // 2, v.shape[0] // 2), pl.ds(c0, v.shape[1]))] = _pack(v)


LEFT = ((1, 4), (3, 4), (1,), (4,), (1, 2), (3, -1), (2, -4))
RIGHT = ((1, 4), (1,), (2, -4), (3, -1), (4,), (1, 2), (3, 4))
OUT = ((1, 4, -5, 7), (3, 5), (2, 4), (1, -2, 3, 6))
LEFT_T = ((1, -4), (3, -4), (2, -4), (3, -1), (1, -2), (4,), (1,))
OUT_T = ((1, 6, -5, 3), (7, -5), (2, 6), (2, -1, 7, 4))


def _sum(terms, get):
    v = get(terms[0] - 1)
    for term in terms[1:]:
        v = v + get(term - 1) if term > 0 else v - get(-term - 1)
    return v


def _sums(scheme, xs):
    return [_sum(terms, lambda n: xs[n]) for terms in scheme]


def _sum2(scheme, outer, inner, get):
    return _sum(scheme[outer], lambda a: _sum(scheme[inner], lambda b: get(a, b)))


def _sums2(scheme, outer, get):
    return _sums(scheme, [_sum(scheme[outer], lambda a: get(a, b)) for b in range(4)])


_aset = lambda *x: _sums(LEFT, x)
_bset = lambda *x: _sums(RIGHT, x)
_tset = lambda *x: _sums(LEFT_T, x)
_post = lambda m: _sums(OUT, m)


def _weave(main, *sides):
    main = [f for item in main for f in (item if isinstance(item, list) else [item])]
    done = [0] * len(sides)
    if not main:
        return
    for n, item in enumerate(main):
        v = item()
        for s, (pace, side) in enumerate(sides):
            upto = (n + 1) * len(side) // len(main)
            if done[s] < upto and v is not None and pace is not None:
                pace(v())
            while done[s] < upto:
                side[done[s]]()
                done[s] += 1


def _ride(main, *sides):
    main = [f for item in main for f in (item if isinstance(item, list) else [item])]
    keep = len(main) - max(1, len(main) // 6)
    _weave(main[:keep], *sides)
    _weave(main[keep:])


def _kernel(xT_hbm, gT_hbm, wqkv_hbm, wo_hbm, w1_hbm, w2T_hbm, b1_ref, b2_ref,
            outT_hbm, dxT_hbm, dwqkv_hbm, dwo_hbm, dw1_hbm, db1_ref, dw2T_hbm, db2_ref,
            xb, gb, wqkv_b, wo_b, w_b, dw_b, acc_w, stats, outM, dyM, qkv, oT, dT, db1_s, zero_s, sem_in, sem_w, sem_out):

    def tile_in(src, dst, i, s):
        return pltpu.make_async_copy(src.at[:, pl.ds(i * TS, TS)], dst.at[i, pl.ds(0, D)], sem_in.at[s])

    cp_g = [tile_in(gT_hbm, gb, i, i) for i in range(NT)]
    cp_x = [tile_in(xT_hbm, xb, i, NT + i) for i in range(NT)]
    cp_wo = pltpu.make_async_copy(wo_hbm, wo_b, sem_in.at[2 * NT])
    cp_wqkv = pltpu.make_async_copy(wqkv_hbm, wqkv_b.at[0, pl.ds(0, D)], sem_in.at[2 * NT + 1])

    def cols(j):
        return pl.ds(j * FC if isinstance(j, int) else pl.multiple_of(j * FC, FC), FC)

    def cp_w(j, n):
        slot = n * RING + (j & RING - 1)
        return pltpu.make_async_copy((w1_hbm, w2T_hbm)[n].at[:, cols(j)], w_b.at[slot, pl.ds(0, D)], sem_w.at[slot])

    def cp_dw(j, n):
        slot = 2 * n + (j & 1)
        return pltpu.make_async_copy(dw_b.at[slot], (dw1_hbm, dw2T_hbm)[n].at[:, cols(j)], sem_w.at[2 * RING + slot])

    for c in (cp_wo, cp_g[0]):
        c.start()
    zero_s[0] = 0
    tie = {"z": zero_s[0]}

    def pacer(*refs, slab=0):
        def pace(v):
            for ref in refs:
                w = pltpu.bitcast(v, ref.dtype)
                rows = pl.ds(ref.shape[-2] - w.shape[0], w.shape[0])
                ref[(tie["z"] + slab,) + (0,) * (len(ref.shape) - 3) + (rows, slice(0, L))] = w
        return pace

    def probe(ref, first, r0=0):
        return lambda: ref[tie["z"] + first, pl.ds(r0, 8), pl.ds(0, L)]

    def fenced(main, sides, stops, gate, written):
        legs = [(lo, hi, free) for lo, (hi, free) in zip([0] + [f for _, f in stops], stops)]
        span, done = sum(hi - lo for lo, hi, _ in legs), 0
        for lo, hi, free in legs:
            _weave(main[lo:hi], *[cut(v, done / span, (done + hi - lo) / span) for v in sides])
            _weave(main[hi:free])
            done += hi - lo
            for src in written:
                m = 16 if src.dtype == bf16 else 8
                gate(src[tie["z"], pl.ds(pl.multiple_of(tie["z"], m), m), 0:L])
        _weave(main[stops[-1][1]:])

    def block(body):
        pl.when(tie["z"] == 0)(body)

    def segments(product, rows, store):
        n, held = rows // 4, {}

        def segment(r):
            def run():
                if r == 0:
                    held[0] = product()
                return store(held[0][n * r:n * (r + 1)], pl.ds(n * r, n))
            return run
        return [segment(r) for r in range(4)]

    def cut(stream, a, b):
        pace, todo = stream
        return pace, todo[int(len(todo) * a):int(len(todo) * b)]

    def aligned(v, m):
        return v if isinstance(v, int) else pl.multiple_of(v, m)

    def finish_dw(j, quarter):
        n, r0 = quarter >> 1, aligned((quarter & 1) * (DQ // 2), 8)
        acc = acc_w.at[0, pl.ds(aligned(STACK * (2 * (j & 1) + n), 1024), STACK)]

        def piece(r, b):
            def run():
                parts = [_sum(OUT[b], lambda m: acc[pl.ds(r0 + (DQ * (7 * k + m) + 8 * r), 8)]) for k in range(7)]
                for a, v in enumerate(_sums(OUT, parts)):
                    dw_b[2 * n + (j & 1), pl.ds(r0 + (DH * (a // 2) + DQ * (b // 2) + 8 * r), 8),
                         pl.ds(FH * (a % 2) + L * (b % 2), L)] = v.astype(bf16)
            return run
        return pacer(acc_w), [piece(r, b) for r in range(DQ // 16) for b in range(4)]

    def normed(x, i, c, twice):
        m1, r1, m2, r2 = [stats[i, n, :, pl.ds(L * c, L)] for n in range(4)]
        xn = (x - m1) * r1
        return (xn - m2) * r2 if twice else xn

    def main_phases(ya, ga, yTa, gTa, wB, b1_s):
        def right_w(j, quarter):
            n, r0 = quarter >> 1, aligned((quarter & 1) * L, L)
            src, dst = w_b.at[n * RING + (j & RING - 1)], wB.at[pl.ds(7 * (2 * (j & 1) + n), 7)]

            def piece(r):
                def run():
                    q = lambda a, c: _unpack(src[pl.ds(r0 + (256 * a + 16 * r), 16), c * FH:(c + 1) * FH])
                    for k, v in enumerate(_bset(q(0, 0), q(0, 1), q(1, 0), q(1, 1))):
                        dst[k, pl.ds(aligned(r0 >> 1, 8) + 8 * r, 8)] = _pack(v)
                return run

            def tail():
                for k, c in ((2, 1), (3, 0), (5, 1), (6, 0)):
                    dst[k, 128:160] = pltpu.bitcast(src[512:576, c * FH:(c + 1) * FH], u32)
                    rows = jax.lax.broadcasted_iota(jnp.int32, (16, FH), 0)
                    b = jnp.broadcast_to(b1_s[j, :, c * FH:(c + 1) * FH], (16, FH))
                    dst[k, 160:168] = _pack(jnp.where(rows < 1 - n, b, 0.0))
            return pacer(w_b), [piece(r) for r in range(L // 16)] + [tail]

        def source(is_x, twice):
            def get(i, r0, n, c, unpack=_unpack):
                v = unpack((xb if is_x else gb)[i, pl.ds(r0, n), pl.ds(L * c, L)])
                return normed(v, i, c, twice) if is_x else v
            return get

        def combos_T(get, dst, i, r):
            st = {}

            def load():
                for a in range(4):
                    for b in range(4):
                        st[a, b] = get(i, DH * (a // 2) + DQ * (b // 2) + 16 * r, 16, 2 * (a % 2) + b % 2)

            def sums(k):
                def run():
                    for n, v in enumerate(_sums2(LEFT, k, lambda a, b: st[a, b])):
                        _st(dst, (0,), STACK * i + DQ * (7 * k + n) + 16 * r, v)
                return run
            return [load] + [sums(k) for k in range(7)]

        def prologue(wP, xB, nat):
            def norm(i, c):
                cs = pl.ds(L * c, L)
                stat = lambda n: stats[i, n, :, cs]
                terms = (lambda x: x, lambda x: jnp.square(x - stat(0)), lambda x: (x - stat(0)) * stat(1),
                         lambda x: jnp.square((x - stat(0)) * stat(1) - stat(2)))

                def sweep(n):
                    def run():
                        total = 0.0
                        for r in range(0, D, 64):
                            v = terms[n](_unpack(xb[i, pl.ds(r, 64), cs]))
                            total = total + sum(v[8 * m:8 * m + 8] for m in range(1, 8)) + v[0:8]
                        mean = jnp.sum(total, 0, keepdims=True) * (1.0 / D)
                        stats[i, n, :, cs] = jax.lax.rsqrt(mean + EPS) if n % 2 else mean
                    return run
                return [sweep(n) for n in range(4)]

            def flip(get, i, c, r, fill):
                def run():
                    n = min(L, D - L * r)
                    v = get(i, L * r, n, c, lambda w: w.astype(f32))
                    if n < L:
                        row = jax.lax.broadcasted_iota(jnp.int32, (L - n, L), 0)
                        v = jnp.concatenate([v, jnp.where(row == 0, fill, 0.0)], 0)
                    nat[r, pl.ds(L * c, L)] = v.T
                return run

            def wide_aset(q):
                blocks = (q(0, 0, 2), q(0, 2, 2), q(1, 0, 2), q(1, 2, 2))
                t1, t2 = q(0, 4, 1), q(1, 4, 1)
                tails = {2: t1, 3: t2, 5: t2 - t1, 6: t1 - t2}
                return [jnp.concatenate([v, tails[k]], 1) if k in tails else v
                        for k, v in enumerate(_aset(*blocks))], blocks, t1 + t2

            def combos_N(dst, i, r, is_g):
                def run():
                    q = lambda half, c0, n: jnp.concatenate(
                        [_split(nat, (c0 + u,), TH * half + 16 * r, 16) for u in range(n)], 1)
                    vs, blocks, tail = wide_aset(q)
                    for k, v in enumerate(vs):
                        _st(dst, (7 * i + k,), 16 * r, v)
                    if is_g:
                        t = jnp.concatenate([blocks[0] + blocks[2], blocks[1] + blocks[3], tail], 1)
                        t = t[0:8] + t[8:16]
                        db1_s[NF] += t[:, 0:FC]
                        db1_s[NF + 1, :, 0:L] += t[:, FC:DP]
                return run

            def layouts(i, is_x):
                get = source(is_x, True)
                return ([flip(get, i, c, r, 1.0 if is_x else 0.0) for c in range(4) for r in range(5)] +
                        [f for r in range(DQ // 16 if is_x else 0) for f in combos_T(get, yTa, i, r)] +
                        [combos_N(ya if is_x else ga, i, r, not is_x) for r in range(TH // 16)])

            def right(i):
                def piece(r, c):
                    return lambda: _st(xB, (i % 2,), 64 * r, source(True, False)(i, 64 * r, 64, c), L * c)
                return [piece(r, c) for r in range(D // 64) for c in range(4)]

            def put_left(part, r, v):
                for e in range(2):
                    wP[part, pl.ds(DH * e + 16 * r, 16), :] = v[16 * e:16 * (e + 1), 0:D].astype(bf16)

            def flip_w(c, r):
                def run():
                    n, m = min(L, 3 * D - L * c), min(L, D - L * r)
                    v = wqkv_b[0, pl.ds(L * r, m), pl.ds(L * c, n)].astype(f32)
                    if n < L:
                        v = jnp.concatenate([v, jnp.zeros((m, L - n), f32)], 1)
                    if m < L:
                        v = jnp.concatenate([v, jnp.zeros((L - m, L), f32)], 0)
                    nat[r, pl.ds(TS + L * c, L)] = v.T
                return run

            def left_w(part):
                def piece(r):
                    return lambda: put_left(part, r, jnp.concatenate(
                        [_split(nat, (u,), TS + D * part + 32 * r, 32) for u in range(5)], 1))
                return [piece(r) for r in range(D // 32)]

            def project(i, part):
                def item(c, e):
                    rows, cs, n = pl.ds(DQ * e, DQ), pl.ds(TH * c, TH), DQ // 3

                    def segment(r, held):
                        def run():
                            if r == 0:
                                rhs = gb[i, 0:D, cs] if part == 3 else _ld(xB, (i % 2,), cols=cs)
                                held.append(_dot(jnp.concatenate(
                                    [wP[part, pl.ds(DH * u + DQ * e, DQ), :] for u in range(2)], 0), rhs))
                            v = jnp.concatenate([held[0][DQ * u + n * r:DQ * u + n * (r + 1)] for u in range(2)], 0)
                            at = DH * part + DQ * e + n * r
                            for u in range(2):
                                qkv[4 * i + 2 * c + u + 1, pl.ds(at, n)] = _pack(v[:, L * u:L * (u + 1)])
                            return probe(qkv, 4 * i + 2 * c + 1, at)
                        return run
                    held = []
                    return [segment(r, held) for r in range(3)]
                return [item(c, e) for c in range(2) for e in range(2)]

            def setup():
                b = b1_ref[...].astype(f32).reshape(1, F)
                for j in range(NF):
                    b1_s[j] = b[:, FC * j:FC * (j + 1)]
                for k in range(28):
                    wB[k, 160:192, :] = jnp.zeros((32, FH), u32)
                db1_s[...] = jnp.zeros(db1_s.shape, f32)
                for t in (0, NL + 1):
                    qkv[t] = jnp.zeros(qkv.shape[1:], u32)

            later = [cp_g[1], cp_wqkv, cp_x[0], cp_g[2], cp_g[3], cp_x[1], cp_x[2], cp_x[3]]
            later += [cp_w(j, n) for j in range(3) for n in range(2)]
            for c in later[:3]:
                c.start()
            setup()
            cp_wo.wait()
            for r in range(D // 32):
                put_left(3, r, _unpack(wo_b[pl.ds(32 * r, 32), :]))
            cp_g[0].wait()
            pg, px, pw = pacer(gb), pacer(xb), pacer(nat)

            flips = [flip_w(c, r) for c in range(14) for r in range(5)]

            def job(i, part):
                stats_of = lambda m: (px, [f for c in range(4) for f in norm(m, c)] + right(m))
                if part == 3:
                    sides = ([(pg, layouts(0, False))], [(pw, flips[:35])], [(pw, flips[35:])],
                             [stats_of(0), (pw, left_w(0))])[i]
                else:
                    sides = [(pw, left_w(part + 1))] if i == 0 and part < 2 else []
                    if part == 0 and i > 0:
                        sides.append((pg, layouts(i, False)))
                    if part > 0:
                        todo = layouts(i, True)
                        sides.append((px, todo[:20] + todo[-16:] if part == 1 else todo[20:-16]))
                    if part == 2:
                        sides += [stats_of(i + 1)] if i + 1 < NT else [right_w(0, m) for m in range(4)]
                _ride(project(i, part), *sides)

            for i in range(NT):
                for c in later[3 + 2 * i:5 + 2 * i]:
                    c.start()
                (cp_g[i + 1] if i + 1 < NT else cp_x[0]).wait()
                if i == 1:
                    cp_wqkv.wait()
                block(lambda: job(i, 3))
            for c in later[11:]:
                c.start()
            for i in range(NT):
                for part in range(3):
                    if part == 2:
                        for c in [cp_x[i + 1]] if i + 1 < NT else later[8:12]:
                            c.wait()
                    block(lambda: job(i, part))

        pl.run_scoped(prologue,
                      pltpu.VMEM((4, D, D), bf16), pltpu.VMEM((2, *_words(D, TS)), u32),
                      pltpu.VMEM((5, TS + 14 * L + 8, L), f32))

        def mlp(wA, mp, md, hB, dB, p_s, dl_s, hd_s):
            tie["z"] = zero_s[0]

            def left_w(j, quarter):
                n, r0 = quarter >> 1, aligned((quarter & 1) * 64, 64)
                src, dst = w_b.at[n * RING + (j & RING - 1)], wA.at[0, pl.ds(aligned(STACK // 2 * (2 * (j & 1) + n), 512), STACK // 2)]

                def piece(r, k):
                    def run():
                        q = lambda a, b: _unpack(src[pl.ds(r0 + (DH * (a // 2) + DQ * (b // 2) + 16 * r), 16),
                                                     pl.ds(FH * (a % 2) + L * (b % 2), L)])
                        for m, v in enumerate(_sums2(LEFT_T, k, q)):
                            dst[pl.ds(aligned(r0 >> 1, 8) + (DQ // 2 * (7 * k + m) + 8 * r), 8)] = _pack(v)
                    return run
                return pacer(w_b), [piece(r, k) for r in range(5) for k in range(7)]

            def stage_A(n):
                i, j = n & 3, n >> 2

                def item(xa, w, m, k):
                    def store(v, rows):
                        m[2 * k, rows] = v[:, 0:L]
                        m[2 * k + 1, rows] = v[:, L:FH]
                        return probe(m, 2 * k)
                    return segments(lambda: _dot(_ld(xa, (7 * i + k,), cols=slice(0, KW[k])),
                                                 _ld(wB, (7 * (2 * (j & 1) + w) + k,), 0, KW[k])), TH, store)
                return [item(ya, 0, mp, k) for k in range(7)] + [item(ga, 1, md, k) for k in range(7)]

            def stage_G(n):
                def piece(r, c):
                    st = {}

                    def total(m, e):
                        return _post([m[2 * k + c, pl.ds(16 * r + e, 8, stride=2)] for k in range(7)])

                    def act(e):
                        def run():
                            st["h", e], st["g"] = [], []
                            for p in total(mp, e):
                                p2 = p * p
                                a = 0.5 + 0.5 * jnp.tanh(p * (C0 + (C0 * C1) * p2))
                                h = p * a
                                st["h", e].append(h)
                                st["g"].append(a + (h - h * a) * (2 * C0 + (6 * C0 * C1) * p2))
                            if e == 1:
                                emit(hB, "h")
                        return run

                    def grad(e):
                        def run():
                            st["d", e] = [d * g for d, g in zip(total(md, e), st["g"])]
                            if e == 1:
                                emit(dB, "d")
                                for half in range(2):
                                    t = (st["d", 0][half] + st["d", 0][2 + half]) + (st["d", 1][half] + st["d", 1][2 + half])
                                    where = pl.ds(half * FH + L * c, L)
                                    db1_s[n >> 2, :, where] += t
                        return run

                    def emit(dst, name):
                        for q, v in enumerate(zip(st[name, 0], st[name, 1])):
                            at = (r % 8, "hd".index(name), 2 * (r // 8) + c, q)
                            hd_s[at] = jnp.concatenate(v, 0)
                    return [act(0), grad(0), act(1), grad(1)]

                def second(r, w, k):
                    def run():
                        for m, v in enumerate(_sums2(RIGHT, k, lambda a, b: hd_s[r, w, b, a])):
                            _st((hB, dB)[w], (7 * k + m,), 16 * r, v)
                    return run
                return ((pacer(mp, md),
                         [f for r in range(TH // 16) for c in range(2) for f in piece(r, c)]),
                        (pacer(hd_s, slab=8), [second(r, w, k) for w in range(2) for r in range(L // 16) for k in range(7)]))

            def stage_BC(n):
                i, j = n & 3, n >> 2
                plan = (((acc_w, 2 * (j & 1) + 1), i > 0, (gTa, i), hB, _NN),
                        ((acc_w, 2 * (j & 1)), i > 0, (yTa, i), dB, _NN),
                        ((outM, i), j > 0, (wA, 2 * (j & 1) + 1), hB, _NT),
                        ((dyM, i), j > 0, (wA, 2 * (j & 1)), dB, _NT))
                jobs = [(*p, k) for p in plan for k in range(49)]

                def group(four):
                    m, held = DQ // 3, []

                    def segment(r):
                        def run():
                            if r == 0:
                                held.extend(_dot(pltpu.bitcast(a[0, pl.ds(aligned(STACK // 2 * at, 512) + DQ // 2 * k, DQ // 2)], bf16), _ld(b, (k,), 0, L), dims)
                                            for _, _, (a, at), b, dims, k in four)
                            old = [jnp.where(started, acc[0, pl.ds(aligned(STACK * at, 1024) + (DQ * k + m * r), m)], 0.0)
                                   for (acc, at), started, *_, k in four]
                            for ((acc, at), *_, k), u, v in zip(four, old, held):
                                acc[0, pl.ds(aligned(STACK * at, 1024) + (DQ * k + m * r), m)] = u + v[m * r:m * (r + 1)]
                            return probe(acc, 0, aligned(STACK * at, 1024) + DQ * k)
                        return run
                    return [segment(r) for r in range(3)]
                return [group(jobs[k:k + 4]) for k in range(0, len(jobs), 4)]

            def attention(t, hg):
                st = {}
                lane = lambda: jax.lax.broadcasted_iota(jnp.int32, (8, L), 1)

                def rows(part, d):
                    return pl.ds((part * D + 8 * HD * hg) // 2 + d, 8, stride=HD // 2)

                def ld(dt, part, d):
                    return qkv[t + 1 + dt, rows(part, d), :]

                def back(cur, prev, w):
                    if w == 0:
                        return cur
                    return pltpu.roll(jnp.where(lane() < L - DIL * w, cur, prev), DIL * w, 1)

                def ahead(cur, nxt, w):
                    if w == 0:
                        return cur
                    return pltpu.roll(jnp.where(lane() >= DIL * w, cur, nxt), L - DIL * w, 1)

                def scores(own, other, dst, d):
                    def run():
                        a, cur, prev = _unpack(ld(0, own, d)), ld(0, other, d), ld(-1, other, d)
                        for w in range(W):
                            v = a * _unpack(back(cur, prev, w))
                            v = v[0:8] + v[8:16]
                            st[w] = v if d == 0 else st[w] + v
                            if d == HD // 2 - 1:
                                dst[t & 3, hg, w] = st[w]
                    return run

                def soft():
                    pos = lane() + t * L
                    lg = [jnp.where(pos >= DIL * w, p_s[t & 3, hg, w] * HD ** -0.5, -1e9) for w in range(W)]
                    m = lg[0]
                    for w in range(1, W):
                        m = jnp.maximum(m, lg[w])
                    e = [jnp.exp(x - m) for x in lg]
                    tot = e[0]
                    for w in range(1, W):
                        tot = tot + e[w]
                    inv = 1.0 / tot
                    p = [x * inv for x in e]
                    dp = [dl_s[t & 3, hg, w] for w in range(W)]
                    c = p[0] * dp[0]
                    for w in range(1, W):
                        c = c + p[w] * dp[w]
                    for w in range(W):
                        p_s[t & 3, hg, w] = p[w]
                        dl_s[t & 3, hg, w] = jnp.where(pos >= DIL * w, p[w] * (dp[w] - c) * HD ** -0.5, 0.0)

                def gather(src, other, dst, part, d):
                    def run():
                        if d == 0:
                            for w in range(W):
                                st[w] = jnp.concatenate([src[t & 3, hg, w]] * 2, 0)
                        cur, prev = ld(0, other, d), ld(-1, other, d)
                        v = st[0] * _unpack(cur)
                        for w in range(1, W):
                            v = v + st[w] * _unpack(back(cur, prev, w))
                        dst[t, rows(part, d), :] = _pack(v)
                    return run

                def scatter(src, other, dst, part, d):
                    def run():
                        if d == 0:
                            for w in range(W):
                                st[w] = jnp.concatenate([ahead(src[t & 3, hg, w], src[(t + 1) & 3, hg, w], w)] * 2, 0)
                        cur, nxt = ld(0, other, d), ld(1, other, d)
                        v = st[0] * _unpack(cur)
                        for w in range(1, W):
                            v = v + st[w] * _unpack(ahead(cur, nxt, w))
                        dst[t, rows(part, d), :] = _pack(v)
                    return run

                ds = range(HD // 2)
                return ([scores(0, 1, p_s, d) for d in ds] + [scores(3, 2, dl_s, d) for d in ds] + [soft] +
                        [gather(p_s, 2, oT, 0, d) for d in ds] + [gather(dl_s, 1, dT, 0, d) for d in ds] +
                        [scatter(dl_s, 0, dT, 1, d) for d in ds] + [scatter(p_s, 3, dT, 2, d) for d in ds])

            for ref in (p_s, dl_s):
                ref[0] = jnp.zeros(ref.shape[1:], f32)

            def wipe(k):
                def run():
                    acc_w[0, pl.ds(STACK * (2 + k // 49) + DQ * (k % 49), DQ)] = jnp.zeros((DQ, L), f32)
                return run
            rows_g = lambda tiles: (pacer(gb), [f for i in tiles for r in range(DQ // 16)
                                                for f in combos_T(source(False, False), gTa, i, r)])
            block(lambda: _ride(stage_A(0), *[left_w(0, m) for m in range(4)], rows_g((0, 1))))

            block(lambda: _weave(stage_G(0)[0][1], (None, rows_g((2,))[1])))
            block(lambda: _ride(stage_A(1), stage_G(0)[1], right_w(1, 0), rows_g((3,)),
                                 (pacer(hB), [wipe(k) for k in range(98)])))

            def step(n, carry):
                tie["z"] = zero_s[0]
                i, j = n & 3, n >> 2

                @pl.when(i == NT - 1)
                def _():
                    for w in range(2):
                        pl.when(j >= 2)(lambda: cp_dw(j - 2, w).wait())
                        pl.when(j + 2 < NF)(lambda: cp_w(j + 2, w).wait())
                        pl.when(j + 3 < NF)(lambda: cp_w(j + 3, w).start())

                @pl.when((i == 0) & (j >= 2))
                def _():
                    for w in range(2):
                        cp_dw(j - 2, w).start()

                m = jnp.minimum(n, 2 * NL - 2 + (n & 1))
                att = (pacer(qkv), [f for u in range(2) for f in attention(NL - 1 - (m >> 1), 2 * (m & 1) + u)])
                g, x = stage_G(n + 1), 0.9
                main = stage_BC(n)
                _weave(main[:-1], g[0], cut(att, 0, x),
                       right_w(jnp.minimum(((n + 1) >> 2) + 1, NF - 1), (n + 1) & 3))
                _weave(main[-1:])
                sides = [g[1], cut(att, x, 1), left_w(jnp.minimum(j + 1, NF - 1), i), finish_dw(j + 1, i)]
                fenced(stage_A(n + 2), sides, ((5, 7), (10, 12)), pacer(ga, slab=NT * 7), (oT, dT, wA, hB, dB, dw_b))
                return carry

            jax.lax.fori_loop(0, NT * NF - 2, step, 0)
            tie["z"] = zero_s[0]


            def drain():
                n = NT * NF - 2
                main, g = stage_BC(n), stage_G(n + 1)
                _weave(main[:40], g[0], finish_dw(NF - 2, 2))
                _weave(main[40:])
                for f in cut(g[1], 0, 0.5)[1]:
                    f()
                main = stage_BC(n + 1)
                _weave(main[:10], cut(g[1], 0.5, 1))
                _weave(main[10:], finish_dw(NF - 2, 3))
            block(drain)
            for w in range(2):
                cp_dw(NF - 3, w).wait()
                cp_dw(NF - 2, w).start()

        V = pltpu.VMEM
        pl.run_scoped(
            mlp, V((1, *_words(4 * STACK, L)), u32), V((14, TH + 8, L), f32), V((14, TH + 8, L), f32),
            V((49, *_words(L + 16, L)), u32), V((49, *_words(L, L)), u32),
            V((4, 4, W, 8, L), f32), V((4, 4, W, 8, L), f32), V((9, 2, 4, 4, 16, L), f32))

    V = pltpu.VMEM
    pl.run_scoped(
        main_phases,
        V((NT * 7 + 1, *_words(TH, 384)), u32), V((NT * 7 + 1, *_words(TH, 384)), u32),
        V((1, *_words(NT * STACK, L)), u32), V((1, *_words(NT * STACK, L)), u32),
        V((4 * 7, *_words(384, FH)), u32), V((NF, 1, FC), f32))

    def epilogue(out_b, dx_b, woT, b2c, wT, xA, dS, fin, work, dwo, *accs):
        tie["z"] = zero_s[0]

        def tile_out(src, dst, i, s):
            return pltpu.make_async_copy(src.at[i], dst.at[:, pl.ds(i * TS, TS)], sem_out.at[s])

        cp_out = [tile_out(out_b, outT_hbm, i, i) for i in range(NT)]
        cp_dx = [tile_out(dx_b, dxT_hbm, i, NT + i) for i in range(NT)]
        cp_dwqkv = [pltpu.make_async_copy(wqkv_b.at[0, pl.ds(0, D), pl.ds(c, n)], dwqkv_hbm.at[:, pl.ds(c, n)],
                                          sem_out.at[2 * NT + 1 + m])
                    for m, (c, n) in enumerate(((0, 3 * TH), (3 * TH, 3 * D - 3 * TH)))]
        cp_dwo = pltpu.make_async_copy(wo_b, dwo_hbm, sem_out.at[2 * NT])

        def wide(ref, t, tiles, r0=0, n=None):
            return jnp.concatenate([_ld(ref, (t + u,), r0, n) for u in range(tiles)], 1)

        def flip_wo(c):
            n = min(L, D - L * c)
            v = wo_b[:, pl.ds(L * c, n)].astype(f32)
            b = b2_ref[...].astype(f32).reshape(1, D)[:, L * c:L * c + n]
            if n < L:
                v = jnp.concatenate([v, jnp.zeros((D, L - n), f32)], 1)
                b = jnp.concatenate([b, jnp.zeros((1, L - n), f32)], 1)
            v = jnp.concatenate([v, jnp.zeros((DP - D, L), f32)], 0)
            woT[pl.ds(L * c, n), :] = v.T[0:n, 0:D].astype(bf16)
            b2c[pl.ds(L * c, n), :] = jnp.broadcast_to(b, (L, L)).T[0:n]

        def left_w(r):
            def run():
                def q(half, c):
                    w = min(QH, 3 * D - QH * c)
                    v = _unpack(wqkv_b[0, pl.ds(DH * half + 16 * r, 16), pl.ds(QH * c, w)])
                    return v if w == QH else jnp.concatenate([v, jnp.zeros((16, QH - w), f32)], 1)
                for k, v in enumerate(_tset(q(0, 0), q(0, 1), q(1, 0), q(1, 1))):
                    _st(wT, (k,), 16 * r, v)
            return run

        def left_x(i, r, u):
            def run():
                q = lambda r0, c: normed(_unpack(xb[i, pl.ds(r0 + 48 * r, 48), pl.ds(L * (2 * c + u), L)]),
                                         i, 2 * c + u, False)
                for k, v in enumerate(_aset(q(0, 0), q(0, 1), q(DH, 0), q(DH, 1))):
                    _st(xA, (k,), 48 * r, v, TH * i + L * u)
            return run

        def right_d(i, r, u):
            def run():
                def q(half, c):
                    if QH * half + 32 * r >= 3 * D:
                        return jnp.zeros((32, L), f32)
                    return _unpack(dT[4 * i + 2 * c + u, pl.ds((QH * half + 32 * r) // 2, 16)])
                for k, v in enumerate(_bset(q(0, 0), q(1, 0), q(0, 1), q(1, 1))):
                    _st(dS, (k,), 32 * r, v, TH * i + L * u)
            return run

        def rights(i):
            return [right_d(i, r, u) for r in range(QH // 32) for u in range(2)]

        def fwd(i, half, a):
            def store(v, rows):
                fin[half, pl.ds(DH * a + rows.start, rows.size)] = v
                return probe(fin, half)
            return segments(lambda: _dot(woT[pl.ds(DH * a, DH), :], wide(oT, 4 * i + 2 * half, 2)), DH, store)

        def fwd_finish(i, r, b):
            def run():
                parts = [_sum(OUT_T[b], lambda n: outM[0, pl.ds(STACK * i + DQ * (7 * k + n) + 8 * r, 8)]) for k in range(7)]
                for a, v in enumerate(_sums(OUT_T, parts)):
                    rows = pl.ds(DH * (a // 2) + DQ * (b // 2) + 8 * r, 8)
                    cs = pl.ds(TH * (a % 2) + L * (b % 2), L)
                    v = v + fin[a % 2, rows, pl.ds(L * (b % 2), L)] + b2c[rows, :] + xb[i, rows, cs].astype(f32)
                    out_b[i, rows, cs] = v.astype(bf16)
            return run

        def bwd(i, acc):
            def item(k):
                def store(v, rows):
                    acc[k, rows] = v
                    return probe(acc, k)
                return segments(lambda: _dot(_ld(wT, (k,)), _ld(dS, (k,), cols=pl.ds(TH * i, TH))), DH, store)
            return [item(k) for k in range(7)]

        def bwd_finish(i, c, acc):
            cs, st, n = pl.ds(L * c, L), {}, 48
            x = lambda r, twice: normed(xb[i, pl.ds(n * r, n), cs].astype(f32), i, c, twice)
            fold = lambda v: sum(v[8 * m:8 * m + 8] for m in range(1, n // 8)) + v[0:8]
            mean = lambda v: jnp.sum(v, 0, keepdims=True) * (1.0 / D)

            def tally(r, name, d, xn):
                work[c % 2, pl.ds(n * r, n)] = d
                s1, s2 = fold(d), fold(d * xn)
                st[name] = (s1, s2) if r == 0 else (st[name][0] + s1, st[name][1] + s2)
                if n * (r + 1) == D:
                    st[name] = [mean(v) for v in st[name]]

            def first(r):
                a, b, r0 = n * r // DH, n * r % DH // DQ, n * r % DQ
                dy = _sum2(OUT_T, 2 * a + c // 2, 2 * b + c % 2, lambda k, m: dyM[0, pl.ds(STACK * i + DQ * (7 * k + m) + r0, n)])
                tally(r, "y", dy, x(r, True))

            def second(r):
                dy, rs = work[c % 2, pl.ds(n * r, n)], pl.ds(n * r % DH, n)
                d = stats[i, 3, :, cs] * (dy - st["y"][0] - x(r, True) * st["y"][1])
                d = d + _sum(OUT_T[2 * (n * r // DH) + c // 2], lambda k: acc[k, rs, pl.ds(L * (c % 2), L)])
                tally(r, "x", d, x(r, False))

            def third(r):
                rs = pl.ds(n * r, n)
                d = stats[i, 1, :, cs] * (work[c % 2, rs] - st["x"][0] - x(r, False) * st["x"][1])
                dx_b[i, rs, cs] = (d + gb[i, rs, cs].astype(f32)).astype(bf16)
            return [lambda f=f, r=r: f(r) for f in (first, second, third) for r in range(D // n)]

        def grad_w(c, n, acc):
            def item(k):
                def store(v, rows):
                    acc[k, rows, 0:n] = v
                    return probe(acc, k)
                return segments(lambda: _dot(_ld(xA, (k,)), _ld(dS, (k,), c, n), _NT), DH, store)

            def finish(r, u):
                def run():
                    for q, v in enumerate(_post([acc[k, pl.ds(16 * r, 16), pl.ds(u, L)] for k in range(7)])):
                        c0 = QH * (q % 2) + c + u
                        w = min(L, 3 * D - c0)
                        wqkv_b[0, pl.ds(DH * (q // 2) + 16 * r, 16), pl.ds(c0, w)] = v[:, 0:w].astype(bf16)
                return run
            return [item(k) for k in range(7)], (pacer(acc), [finish(r, u) for r in range(18) for u in range(0, n, L)])

        for c in range(5):
            flip_wo(c)
        def tile(i):
            _weave([fwd(i, half, a) for half in range(2) for a in range(2)],
                   (pacer(xb), [left_x(i, r, u) for r in range(6) for u in range(2)]), finish_dw(NF - 1, i),
                   (None, [] if i else [left_w(r) for r in range(DH // 16)] + rights(0)))
            _ride(bwd(i, accs[i]), (pacer(dT), rights(i + 1) if i + 1 < NT else []),
                   (pacer(fin, outM), [fwd_finish(i, r, b) for r in range(DQ // 8) for b in range(4)]))

        for i in range(NT):
            block(lambda: tile(i))
            cp_out[i].start()
        for w in range(2):
            cp_dw(NF - 1, w).start()
        grads = [grad_w(c, min(TH, QH - c), accs[NT + n % 2]) for n, c in enumerate(range(0, QH, TH))]
        for i in range(NT - 1):
            block(lambda: _ride(grads[i][0], *([grads[i - 1][1]] if i else []),
                                 (pacer(accs[i], dyM, work),
                                  [f for c in range(4) for f in bwd_finish(i, c, accs[i])])))
            cp_dx[i].start()

        def grad_wo(i):
            def store(v, rows):
                dwo[0, rows] = dwo[0, rows] + v if i else v
                return probe(dwo, 0)
            return segments(lambda: _dot(wide(oT, 4 * i, 4), gb[i, 0:D], _NT), D, store)

        i = NT - 1
        block(lambda: _ride(grads[i][0] + [grad_wo(0)], grads[i - 1][1],
                             cut((pacer(accs[i], dyM, work),
                                  [f for c in range(4) for f in bwd_finish(i, c, accs[i])]), 0, 0.5)))
        cp_dwqkv[0].start()
        block(lambda: _ride([grad_wo(1), grad_wo(2)], grads[i][1],
                             cut((pacer(accs[i], dyM, work),
                                  [f for c in range(4) for f in bwd_finish(i, c, accs[i])]), 0.5, 1)))
        cp_dx[i].start()
        cp_dwqkv[1].start()
        _weave([grad_wo(3)])
        wo_b[...] = dwo[0, 0:D].astype(bf16)

        cp_dwo.start()

        db1 = [jnp.sum(db1_s[j], 0, keepdims=True) for j in range(NF)]
        db1_ref[...] = jnp.concatenate(db1, 1).astype(bf16).reshape(F)
        db2 = jnp.concatenate([db1_s[NF], db1_s[NF + 1, :, 0:L]], 1)
        db2_ref[...] = jnp.sum(db2, 0, keepdims=True)[:, 0:D].reshape(D).astype(bf16)

        for j in (NF - 2, NF - 1):
            for n in range(2):
                cp_dw(j, n).wait()
        for c in cp_out + cp_dx + cp_dwqkv + [cp_dwo]:
            c.wait()

    pl.run_scoped(epilogue, V((NT, D, TS), bf16), V((NT, D, TS), bf16), V((D, D), bf16), V((D, L), f32),
                  V((7, *_words(DH, QH)), u32), V((7, *_words(DH, NT * TH)), u32), V((7, *_words(QH, NT * TH)), u32),
                  V((2, D + 8, TH), f32), V((2, D + 8, L), f32), V((1, D + 8, D), f32),
                  *[V((7, DH + 8, TH), f32)] * (NT + 2))


@jax.jit
def pallas_parallel_sum__sliding_local_dilated__mixer_channel_mlp__prompt_kernel(
        A_x, A_wqkv, A_wo, B_x, B_w1, B_b1, B_w2, B_b2, grad_out):
    del B_x
    V = pltpu.VMEM
    hbm = pl.BlockSpec(memory_space=pl.ANY)
    vmem = pl.BlockSpec(memory_space=pltpu.VMEM)
    sds = lambda *s: jax.ShapeDtypeStruct(s, bf16)
    outT, dxT, dwqkv, dwo, dw1, db1, dw2T, db2 = pl.pallas_call(
        _kernel,
        in_specs=[hbm] * 6 + [vmem] * 2,
        out_specs=[hbm] * 5 + [vmem, hbm, vmem],
        out_shape=[sds(D, S), sds(D, S), sds(D, 3 * D), sds(D, D), sds(D, F), sds(F), sds(D, F), sds(D)],
        scratch_shapes=[
            V((NT, D + 16, TS), bf16), V((NT, D + 16, TS), bf16), V((1, D + 16, 3 * D), bf16), V((D, D), bf16),
            V((2 * RING, D + 16, FC), bf16), V((4, D, FC), bf16), V((1, 4 * STACK, L), f32), V((NT, 4, 1, TS), f32),
            V((1, NT * STACK, L), f32), V((1, NT * STACK, L), f32), V((NL + 2, *_words(4 * D + 16, L)), u32),
            V((NL, *_words(D, L)), u32), V((NL, *_words(3 * D + 16, L)), u32),
            V((NF + 2, 8, FC), f32), pltpu.SMEM((2,), jnp.int32),
            pltpu.SemaphoreType.DMA((2 * NT + 2,)), pltpu.SemaphoreType.DMA((2 * RING + 4,)),
            pltpu.SemaphoreType.DMA((2 * NT + 3,)),
        ],
        compiler_params=pltpu.CompilerParams(vmem_limit_bytes=127 * 2**20),
    )(A_x[0].T, grad_out[0].T, A_wqkv, A_wo, B_w1, B_w2.T, B_b1, B_b2)
    return (outT.T[None], dxT.T[None], dwqkv, dwo, dw1, db1, dw2T.T, db2)
```
